```python
import jax
import jax.numpy as jnp

def _softmax(x, axis=-1):
    return jax.nn.softmax(x, axis=axis)

def _gelu(x):
    return jax.nn.gelu(x, approximate=True)

def _silu(x):
    return jax.nn.silu(x)

def _sigmoid(x):
    return jax.nn.sigmoid(x)

def _layernorm(x, axis=-1, eps=1e-05):
    m = jnp.mean(x, axis=axis, keepdims=True)
    v = jnp.var(x, axis=axis, keepdims=True)
    return (x - m) / jnp.sqrt(v + eps)

def _scatter_add(tgt, idx, src, axis=0):
    return tgt.at[idx].add(src)

def _segment_sum(src, seg, n):
    return jax.ops.segment_sum(src, seg, n)

class _Rng:

    def __init__(self, key):
        self._k = key

    def _next(self):
        self._k, sub = jax.random.split(self._k)
        return sub

    def normal(self, shape):
        return jax.random.normal(self._next(), shape, dtype=jnp.bfloat16)

    def randint(self, lo, hi, shape):
        return jax.random.randint(self._next(), shape, lo, hi, dtype=jnp.int32)

    def uniform(self, shape, lo=0.0, hi=1.0):
        return jax.random.uniform(self._next(), shape, jnp.bfloat16, lo, hi)

    def permutation(self, n):
        return jax.random.permutation(self._next(), n)
kernel_name = 'interleave_layers__memory_aug_recurrent_mem_tr__mixer_s_mlp__prompt'

def setup_inputs():
    _rng = _Rng(jax.random.key(int.from_bytes(__import__("os").urandom(4), "little")))
    _w = lambda a: (lambda t: t.astype(jnp.bfloat16) if jnp.issubdtype(t.dtype, jnp.floating) else t)(jnp.asarray(a))

    def _A_setup():
        B, S, Dm = (1, 2048, 640)
        H, Dh = (32, 192)
        M, seg = (8, 32)
        seg = min(seg, S)
        S = S // seg * seg
        return {'x': _w((lambda *s: _rng.normal(s) * 0.05)(B, S, Dm)), 'mem0': _w((lambda *s: _rng.normal(s) * 0.05)(B, M, Dm)), 'Wq': _w((lambda *s: _rng.normal(s) * 0.05)(Dm, H, Dh) * Dm ** (-0.5)), 'Wk': _w((lambda *s: _rng.normal(s) * 0.05)(Dm, H, Dh) * Dm ** (-0.5)), 'Wv': _w((lambda *s: _rng.normal(s) * 0.05)(Dm, H, Dh) * Dm ** (-0.5)), 'Wo': _w((lambda *s: _rng.normal(s) * 0.05)(H, Dh, Dm) * (H * Dh) ** (-0.5)), 'seg_len': seg}
    _A_in = _A_setup()

    def _B_setup():
        B, S, D, F = (1, 2048, 640, 1536)
        return {'x': _w((lambda *s: _rng.normal(s) * 0.05)(B, S, D)), 'w1': _w((lambda *s: _rng.normal(s) * 0.05)(D, D) * D ** (-0.5)), 'w2': _w((lambda *s: _rng.normal(s) * 0.05)(D, D) * D ** (-0.5)), 'w3': _w((lambda *s: _rng.normal(s) * 0.05)(D, F) * D ** (-0.5)), 'w4': _w((lambda *s: _rng.normal(s) * 0.05)(F, D) * F ** (-0.5))}
    _B_in = _B_setup()
    return {'A_x': _A_in['x'], 'A_mem0': _A_in['mem0'], 'A_Wq': _A_in['Wq'], 'A_Wk': _A_in['Wk'], 'A_Wv': _A_in['Wv'], 'A_Wo': _A_in['Wo'], 'A_seg_len': _A_in['seg_len'], 'B_x': _B_in['x'], 'B_w1': _B_in['w1'], 'B_w2': _B_in['w2'], 'B_w3': _B_in['w3'], 'B_w4': _B_in['w4']}

def reference(A_x, A_mem0, A_Wq, A_Wk, A_Wv, A_Wo, A_seg_len, B_x, B_w1, B_w2, B_w3, B_w4):

    def _A_ref(x, mem0, Wq, Wk, Wv, Wo, seg_len):
        B, S, Dm = x.shape
        H, Dh = (Wq.shape[1], Wq.shape[2])
        M = mem0.shape[1]
        scale = Dh ** (-0.5)
        n_seg = S // seg_len
        L = M + seg_len
        idx = jnp.arange(L)
        mask = (idx[:, None] < M) | (idx[:, None] >= idx[None, :])
        mem = mem0
        outs = []
        for s in range(n_seg):
            xs = x[:, s * seg_len:(s + 1) * seg_len, :].copy()
            h = jnp.concatenate([mem, xs], axis=1)
            q = jnp.einsum('btd,dhe->bhte', h, Wq)
            k = jnp.einsum('btd,dhe->bhte', h, Wk)
            v = jnp.einsum('btd,dhe->bhte', h, Wv)
            scores = jnp.einsum('bhqe,bhke->bhqk', q, k) * scale
            scores = jnp.where(mask[None, None], scores, -1000000000.0)
            p = _softmax(scores, axis=-1)
            o = jnp.einsum('bhqk,bhke->bhqe', p, v)
            o = jnp.einsum('bhte,hed->btd', o, Wo)
            mem = o[:, :M, :].copy()
            outs.append(o[:, M:, :])
        return jnp.concatenate(outs, axis=1)

    def _B_ref(x, w1, w2, w3, w4):
        B, S, D = x.shape
        h = _gelu(_layernorm(x, axis=-1) @ w1)
        c = D // 4
        g0 = jnp.pad(h[:, :, 0 * c:1 * c], ((0, 0), (1, 0), (0, 0)))[:, :S, :]
        g1 = jnp.pad(h[:, :, 1 * c:2 * c], ((0, 0), (0, 1), (0, 0)))[:, 1:, :]
        g2 = jnp.pad(h[:, :, 2 * c:3 * c], ((0, 0), (2, 0), (0, 0)))[:, :S, :]
        g3 = jnp.pad(h[:, :, 3 * c:], ((0, 0), (0, 2), (0, 0)))[:, 2:, :]
        hs = jnp.concatenate([g0, g1, g2, g3], axis=-1) @ w2
        x1 = x + hs
        h2 = _gelu(_layernorm(x1, axis=-1) @ w3) @ w4
        return x1 + h2
    x = A_x
    x = x + _A_ref(_layernorm(x, axis=-1), A_mem0, A_Wq, A_Wk, A_Wv, A_Wo, A_seg_len)
    x = x + _B_ref(_layernorm(x, axis=-1), B_w1, B_w2, B_w3, B_w4)
    x = x + _A_ref(_layernorm(x, axis=-1), A_mem0, A_Wq, A_Wk, A_Wv, A_Wo, A_seg_len)
    x = x + _B_ref(_layernorm(x, axis=-1), B_w1, B_w2, B_w3, B_w4)
    return x
```

```python
import functools
import numpy as np
import jax
import jax.numpy as jnp
from jax import lax
from jax.experimental import pallas as pl
from jax.experimental.pallas import tpu as pltpu

F32 = jnp.float32
BF16 = jnp.bfloat16

S, D, H, DH, M, SEG, FF = 2048, 640, 32, 192, 8, 32, 1536
NSEG = S // SEG
HD = H * DH
NP = H // 2
PW = 2 * DH
LAG = 3
NT_DIMS = (((1,), (1,)), ((), ()))


def _ln(x):
    m = jnp.mean(x, axis=-1, keepdims=True)
    c = x - m
    v = jnp.mean(c * c, axis=-1, keepdims=True)
    return c * lax.rsqrt(v + 1e-5)


def _gelu(x):
    return 0.5 * x * (1.0 + jnp.tanh(0.7978845608028654 * (x + 0.044715 * (x * x * x))))


def kernel(x_hbm, mem0_hbm, wq_hbm, wk_hbm, wv_hbm, wo_hbm, w1_hbm, w2_hbm, w3_hbm, w4_hbm,
           out_hbm,
           x0, mem0, wq, wk, wv, wo, w1, w2, w3, w4,
           xr, hb, ob, lhs, sems, *, gsize):
    srcs = [x_hbm, mem0_hbm, wq_hbm, wk_hbm, wv_hbm, wo_hbm, w1_hbm, w2_hbm, w3_hbm, w4_hbm]
    dsts = [x0, mem0, wq, wk, wv, wo, w1, w2, w3, w4]
    cps = [pltpu.make_async_copy(s, d, sems.at[i]) for i, (s, d) in enumerate(zip(srcs, dsts))]
    for c in cps:
        c.start()
    xr[...] = jnp.zeros(xr.shape, F32)
    hb[...] = jnp.zeros(hb.shape, F32)
    for c in cps:
        c.wait()

    m0 = mem0[...]
    lhs[2 * SEG:2 * SEG + 2 * M, :] = jnp.concatenate([m0, m0], axis=0)

    scale = float(DH) ** -0.5

    def slot(s):
        return jnp.clip(s, -1, NSEG) + 1

    def rows(sl, n=SEG):
        return pl.ds(pl.multiple_of(sl * SEG, SEG), n)

    def step(t, carry):
        r48 = lax.broadcasted_iota(jnp.int32, (48, 96), 0)
        c96 = lax.broadcasted_iota(jnp.int32, (48, 96), 1)
        hi = c96 >= 48
        j = jnp.where(hi, c96 - 48, c96)
        lane128 = lax.broadcasted_iota(jnp.int32, (48, 128), 1)
        lo_l = lane128 < 64

        s1 = t
        s2 = t - LAG
        sl1 = slot(s1)
        sl2 = slot(s2)
        x0s = x0[pl.ds(pl.multiple_of(jnp.minimum(s1, NSEG - 1) * SEG, SEG), SEG), :].astype(F32)
        x2s = xr[rows(sl2), :]
        lhs[0:SEG, :] = _ln(x0s).astype(BF16)
        lhs[SEG:2 * SEG, :] = _ln(x2s).astype(BF16)

        acc = None
        og = []
        for p in range(NP):
            L = lhs[...]
            c0 = p * PW
            q = lax.dot_general(L, wq[c0:c0 + PW, :], NT_DIMS, preferred_element_type=F32).astype(BF16)
            k = lax.dot_general(L, wk[c0:c0 + PW, :], NT_DIMS, preferred_element_type=F32).astype(BF16)
            v = lax.dot_general(L, wv[c0:c0 + PW, :], NT_DIMS, preferred_element_type=F32).astype(BF16)
            outs = []
            for l in range(2):
                ql = jnp.concatenate([q[SEG * l:SEG * l + SEG], q[2 * SEG:]], axis=0)
                kl = jnp.concatenate([k[SEG * l:SEG * l + SEG], k[2 * SEG:]], axis=0)
                vl = jnp.concatenate([v[SEG * l:SEG * l + SEG], v[2 * SEG:]], axis=0)
                z = jnp.zeros((48, 128), BF16)

                def bd(a):
                    a0, a1, a2 = a[:, 0:128], a[:, 128:256], a[:, 256:384]
                    top = jnp.concatenate([a0, jnp.where(lo_l, a1, z), z], axis=1)
                    bot = jnp.concatenate([z, jnp.where(lo_l, z, a1), a2], axis=1)
                    return jnp.concatenate([top, bot], axis=0)

                sc = lax.dot_general(ql, bd(kl), NT_DIMS, preferred_element_type=F32) * scale
                isx = j < 32
                ismem = (j >= 32 + M * l) & (j < 32 + M * l + M)
                allowed = (isx & ((r48 >= 32) | (j <= r48))) | ismem
                fill = jnp.where(isx, -1e9, -jnp.inf).astype(F32)
                sc = jnp.where(allowed, sc, fill)
                m0_ = jnp.max(jnp.where(hi, -jnp.inf, sc), axis=-1, keepdims=True)
                m1_ = jnp.max(jnp.where(hi, sc, -jnp.inf), axis=-1, keepdims=True)
                e = jnp.exp(sc - jnp.where(hi, m1_, m0_))
                d0 = jnp.sum(jnp.where(hi, 0.0, e), axis=-1, keepdims=True)
                d1 = jnp.sum(jnp.where(hi, e, 0.0), axis=-1, keepdims=True)
                pr = (e * jnp.where(hi, 1.0 / d1, 1.0 / d0)).astype(BF16)
                outs.append(jnp.dot(pr, bd(vl), preferred_element_type=F32))
            o = jnp.concatenate([outs[0][0:32], outs[1][0:32], outs[0][32:40], outs[1][40:48]], axis=0).astype(BF16)
            og.append(o)
            if len(og) == gsize:
                g0 = (p + 1 - gsize) * PW
                oc = og[0] if gsize == 1 else jnp.concatenate(og, axis=1)
                r = jnp.dot(oc, wo[g0:g0 + gsize * PW, :], preferred_element_type=F32)
                acc = r if acc is None else acc + r
                og = []

        b1 = t - 1
        b2 = t - LAG - 1
        xin = jnp.concatenate([xr[rows(slot(b1)), :], xr[rows(slot(b1 - LAG)), :]], axis=0)
        zz = _ln(_ln(xin)).astype(BF16)
        h = _gelu(jnp.dot(zz, w1[...], preferred_element_type=F32))
        v1 = (b1 >= 0) & (b1 < NSEG)
        v2 = (b2 >= 0) & (b2 < NSEG)
        hb[0, rows(slot(b1)), :] = jnp.where(v1, h[0:SEG], 0.0)
        hb[1, rows(slot(b2)), :] = jnp.where(v2, h[SEG:], 0.0)

        lane = lax.broadcasted_iota(jnp.int32, (SEG, D), 1)
        parts = []
        for l, sr in enumerate((t - 2, t - LAG - 2)):
            base = pl.multiple_of(slot(sr) * SEG, SEG)
            base = jnp.clip(base, 8, (NSEG + 1) * SEG - 8)
            win = hb[l, pl.ds(pl.multiple_of(base - 8, 8), SEG + 16), :]
            g0 = win[7:7 + SEG]
            g1 = win[9:9 + SEG]
            g2 = win[6:6 + SEG]
            g3 = win[10:10 + SEG]
            parts.append(jnp.where(lane < 320, jnp.where(lane < 160, g0, g1), jnp.where(lane < 480, g2, g3)))
        hc = jnp.concatenate(parts, axis=0).astype(BF16)
        r1 = t - 2
        r2 = t - LAG - 2
        xres = jnp.concatenate([xr[rows(slot(r1)), :], xr[rows(slot(r2)), :]], axis=0)
        y1 = _ln(xres) + jnp.dot(hc, w2[...], preferred_element_type=F32)
        z1 = _ln(y1).astype(BF16)
        h3 = _gelu(jnp.dot(z1, w3[...], preferred_element_type=F32)).astype(BF16)
        xnew = xres + y1 + jnp.dot(h3, w4[...], preferred_element_type=F32)
        xr[rows(slot(r1)), :] = xnew[0:SEG]
        ob[rows(slot(r2)), :] = xnew[SEG:].astype(BF16)

        xr[rows(sl1), :] = x0s + acc[0:SEG]
        xr[rows(sl2), :] = x2s + acc[SEG:2 * SEG]
        mm = acc[2 * SEG:].astype(BF16)
        rr = lax.broadcasted_iota(jnp.int32, (2 * M, D), 0)
        reset = jnp.concatenate([m0, m0], axis=0)
        mm = jnp.where((rr >= M) & (t + 1 <= LAG), reset, mm)
        lhs[2 * SEG:, :] = mm
        return carry

    lax.fori_loop(0, NSEG + LAG + 2, step, 0)
    cp = pltpu.make_async_copy(ob.at[pl.ds(SEG, S)], out_hbm, sems.at[0])
    cp.start()
    cp.wait()


def make(gsize=1):
    def fn(A_x, A_mem0, A_Wq, A_Wk, A_Wv, A_Wo, A_seg_len, B_x, B_w1, B_w2, B_w3, B_w4):
        x = A_x.reshape(S, D)
        mem0 = A_mem0.reshape(M, D)
        tr = lambda w: jnp.transpose(w, (1, 2, 0)).reshape(HD, D)
        wq, wk, wv = tr(A_Wq), tr(A_Wk), tr(A_Wv)
        wo = A_Wo.reshape(HD, D)
        hbm = pl.BlockSpec(memory_space=pltpu.HBM)
        out = pl.pallas_call(
            functools.partial(kernel, gsize=gsize),
            out_shape=jax.ShapeDtypeStruct((S, D), BF16),
            in_specs=[hbm] * 10,
            out_specs=hbm,
            scratch_shapes=[
                pltpu.VMEM((S, D), BF16), pltpu.VMEM((M, D), BF16),
                pltpu.VMEM((HD, D), BF16), pltpu.VMEM((HD, D), BF16), pltpu.VMEM((HD, D), BF16), pltpu.VMEM((HD, D), BF16),
                pltpu.VMEM((D, D), BF16), pltpu.VMEM((D, D), BF16), pltpu.VMEM((D, FF), BF16), pltpu.VMEM((FF, D), BF16),
                pltpu.VMEM(((NSEG + 2) * SEG, D), F32),
                pltpu.VMEM((2, (NSEG + 2) * SEG, D), F32),
                pltpu.VMEM(((NSEG + 2) * SEG, D), BF16),
                pltpu.VMEM((2 * SEG + 2 * M, D), BF16),
                pltpu.SemaphoreType.DMA((10,)),
            ],
            compiler_params=pltpu.CompilerParams(vmem_limit_bytes=110 * 1024 * 1024),
        )(x, mem0, wq, wk, wv, wo, B_w1, B_w2, B_w3, B_w4)
        return out.reshape(1, S, D)
    return fn


_fn = make(gsize=1)


@functools.partial(jax.jit, static_argnames=["A_seg_len"])
def pallas_interleave_layers__memory_aug_recurrent_mem_tr__mixer_s_mlp__prompt_kernel(
        A_x, A_mem0, A_Wq, A_Wk, A_Wv, A_Wo, A_seg_len, B_x, B_w1, B_w2, B_w3, B_w4):
    assert A_seg_len == SEG
    return _fn(A_x, A_mem0, A_Wq, A_Wk, A_Wv, A_Wo, A_seg_len, B_x, B_w1, B_w2, B_w3, B_w4)
```

```python
import functools
import numpy as np
import jax
import jax.numpy as jnp
from jax import lax
from jax.experimental import pallas as pl
from jax.experimental.pallas import tpu as pltpu

F32 = jnp.float32
BF16 = jnp.bfloat16

S, D, H, DH, M, SEG, FF = 2048, 640, 32, 192, 8, 32, 1536
NSEG = S // SEG
HD = H * DH
NP = H // 2
PW = 2 * DH
LAG = 3
NT_DIMS = (((1,), (1,)), ((), ()))


def _ln(x):
    m = jnp.mean(x, axis=-1, keepdims=True)
    c = x - m
    v = jnp.mean(c * c, axis=-1, keepdims=True)
    return c * lax.rsqrt(v + 1e-5)


def _gelu(x):
    return 0.5 * x * (1.0 + jnp.tanh(0.7978845608028654 * (x + 0.044715 * (x * x * x))))


def kernel(x_hbm, mem0_hbm, wq_hbm, wk_hbm, wv_hbm, wo_hbm, w1_hbm, w2_hbm, w3_hbm, w4_hbm,
           out_hbm,
           x0, mem0, wq, wk, wv, wo, w1, w2, w3, w4,
           xr, hb, ob, lhs, sems, *, bh, bh2, bw2, bw3, bw4):
    srcs = [x_hbm, mem0_hbm, wq_hbm, wk_hbm, wv_hbm, wo_hbm, w1_hbm, w2_hbm, w3_hbm, w4_hbm]
    dsts = [x0, mem0, wq, wk, wv, wo, w1, w2, w3, w4]
    cps = [pltpu.make_async_copy(s, d, sems.at[i]) for i, (s, d) in enumerate(zip(srcs, dsts))]
    for c in cps:
        c.start()
    xr[...] = jnp.zeros(xr.shape, F32)
    hb[...] = jnp.zeros(hb.shape, F32)
    for c in cps:
        c.wait()

    m0 = mem0[...]
    lhs[2 * SEG:2 * SEG + 2 * M, :] = jnp.concatenate([m0, m0], axis=0)

    scale = float(DH) ** -0.5

    def slot(s):
        return jnp.clip(s, -1, NSEG) + 1

    def rows(sl, n=SEG):
        return pl.ds(pl.multiple_of(sl * SEG, SEG), n)

    def step(t, carry):
        r48 = lax.broadcasted_iota(jnp.int32, (48, 96), 0)
        c96 = lax.broadcasted_iota(jnp.int32, (48, 96), 1)
        hi = c96 >= 48
        j = jnp.where(hi, c96 - 48, c96)
        lane128 = lax.broadcasted_iota(jnp.int32, (48, 128), 1)
        lo_l = lane128 < 64

        s1 = t
        s2 = t - LAG
        sl1 = slot(s1)
        sl2 = slot(s2)
        x0s = x0[pl.ds(pl.multiple_of(jnp.minimum(s1, NSEG - 1) * SEG, SEG), SEG), :].astype(F32)
        x2s = xr[rows(sl2), :]
        lhs[0:SEG, :] = _ln(x0s).astype(BF16)
        lhs[SEG:2 * SEG, :] = _ln(x2s).astype(BF16)

        def bd(a):
            z = jnp.zeros((48, 128), BF16)
            a0, a1, a2 = a[:, 0:128], a[:, 128:256], a[:, 256:384]
            top = jnp.concatenate([a0, jnp.where(lo_l, a1, z), z], axis=1)
            bot = jnp.concatenate([z, jnp.where(lo_l, z, a1), a2], axis=1)
            return jnp.concatenate([top, bot], axis=0)

        def lrows(a, l):
            return jnp.concatenate([a[SEG * l:SEG * l + SEG], a[2 * SEG:]], axis=0)

        def proj(w, p):
            c0 = p * PW
            return lax.dot_general(lhs[...], w[c0:c0 + PW, :], NT_DIMS, preferred_element_type=F32).astype(BF16)

        def qk(q, k):
            return [lax.dot_general(lrows(q, l), bd(lrows(k, l)), NT_DIMS, preferred_element_type=F32) for l in range(2)]

        def softmax(sc, l):
            sc = sc * scale
            isx = j < 32
            ismem = (j >= 32 + M * l) & (j < 32 + M * l + M)
            allowed = (isx & ((r48 >= 32) | (j <= r48))) | ismem
            fill = jnp.where(isx, -1e9, -jnp.inf).astype(F32)
            sc = jnp.where(allowed, sc, fill)
            m0_ = jnp.max(jnp.where(hi, -jnp.inf, sc), axis=-1, keepdims=True)
            m1_ = jnp.max(jnp.where(hi, sc, -jnp.inf), axis=-1, keepdims=True)
            e = jnp.exp(sc - jnp.where(hi, m1_, m0_))
            d0 = jnp.sum(jnp.where(hi, 0.0, e), axis=-1, keepdims=True)
            d1 = jnp.sum(jnp.where(hi, e, 0.0), axis=-1, keepdims=True)
            return (e * jnp.where(hi, 1.0 / d1, 1.0 / d0)).astype(BF16)

        def pv(prs, v):
            outs = [jnp.dot(prs[l], bd(lrows(v, l)), preferred_element_type=F32) for l in range(2)]
            return jnp.concatenate([outs[0][0:32], outs[1][0:32], outs[0][32:40], outs[1][40:48]], axis=0).astype(BF16)

        def oproj(o, p):
            return jnp.dot(o, wo[p * PW:(p + 1) * PW, :], preferred_element_type=F32)

        b1 = t - 1
        b2 = t - LAG - 1
        r1 = t - 2
        r2 = t - LAG - 2
        st = {}

        def B_h():
            xin = jnp.concatenate([xr[rows(slot(b1)), :], xr[rows(slot(b1 - LAG)), :]], axis=0)
            zz = _ln(_ln(xin)).astype(BF16)
            st['h'] = jnp.dot(zz, w1[...], preferred_element_type=F32)

        def B_h2():
            h = _gelu(st['h'])
            v1 = (b1 >= 0) & (b1 < NSEG)
            v2 = (b2 >= 0) & (b2 < NSEG)
            hb[0, rows(slot(b1)), :] = jnp.where(v1, h[0:SEG], 0.0)
            hb[1, rows(slot(b2)), :] = jnp.where(v2, h[SEG:], 0.0)

        def B_w2():
            lane = lax.broadcasted_iota(jnp.int32, (SEG, D), 1)
            parts = []
            for l, sr in enumerate((r1, r2)):
                base = pl.multiple_of(slot(sr) * SEG, SEG)
                base = jnp.clip(base, 8, (NSEG + 1) * SEG - 8)
                win = hb[l, pl.ds(pl.multiple_of(base - 8, 8), SEG + 16), :]
                g0 = win[7:7 + SEG]
                g1 = win[9:9 + SEG]
                g2 = win[6:6 + SEG]
                g3 = win[10:10 + SEG]
                parts.append(jnp.where(lane < 320, jnp.where(lane < 160, g0, g1), jnp.where(lane < 480, g2, g3)))
            hc = jnp.concatenate(parts, axis=0).astype(BF16)
            st['hs'] = jnp.dot(hc, w2[...], preferred_element_type=F32)

        def B_w3():
            xres = jnp.concatenate([xr[rows(slot(r1)), :], xr[rows(slot(r2)), :]], axis=0)
            y1 = _ln(xres) + st['hs']
            st['y1x'] = xres + y1
            z1 = _ln(y1).astype(BF16)
            st['h3'] = jnp.dot(z1, w3[...], preferred_element_type=F32)

        def B_w4():
            h3 = _gelu(st['h3']).astype(BF16)
            st['h4'] = jnp.dot(h3, w4[...], preferred_element_type=F32)

        def B_out():
            xnew = st['y1x'] + st['h4']
            xr[rows(slot(r1)), :] = xnew[0:SEG]
            ob[rows(slot(r2)), :] = xnew[SEG:].astype(BF16)

        sched = {bh: B_h, bh2: B_h2, bw2: B_w2, bw3: B_w3, bw4: B_w4}
        def fill_at(key):
            for kk, f in ((bh, B_h), (bh2, B_h2), (bw2, B_w2), (bw3, B_w3), (bw4, B_w4)):
                if kk == key:
                    f()

        acc = None
        q = proj(wq, 0); k = proj(wk, 0); v = proj(wv, 0)
        sc = qk(q, k)
        for p in range(NP):
            fill_at(p)
            if p + 1 < NP:
                qn = proj(wq, p + 1)
                kn = proj(wk, p + 1)
            prs = [softmax(sc[0], 0), softmax(sc[1], 1)]
            o = pv(prs, v)
            if p + 1 < NP:
                v = proj(wv, p + 1)
                sc = qk(qn, kn)
            else:
                fill_at(100)
            r = oproj(o, p)
            acc = r if acc is None else acc + r
        fill_at(101)
        B_out()

        xr[rows(sl1), :] = x0s + acc[0:SEG]
        xr[rows(sl2), :] = x2s + acc[SEG:2 * SEG]
        mm = acc[2 * SEG:].astype(BF16)
        rr = lax.broadcasted_iota(jnp.int32, (2 * M, D), 0)
        reset = jnp.concatenate([m0, m0], axis=0)
        mm = jnp.where((rr >= M) & (t + 1 <= LAG), reset, mm)
        lhs[2 * SEG:, :] = mm
        return carry

    lax.fori_loop(0, NSEG + LAG + 2, step, 0)
    cp = pltpu.make_async_copy(ob.at[pl.ds(SEG, S)], out_hbm, sems.at[0])
    cp.start()
    cp.wait()


def make(bh=1, bh2=3, bw2=4, bw3=8, bw4=12):
    def fn(A_x, A_mem0, A_Wq, A_Wk, A_Wv, A_Wo, A_seg_len, B_x, B_w1, B_w2, B_w3, B_w4):
        x = A_x.reshape(S, D)
        mem0 = A_mem0.reshape(M, D)
        tr = lambda w: jnp.transpose(w, (1, 2, 0)).reshape(HD, D)
        wq, wk, wv = tr(A_Wq), tr(A_Wk), tr(A_Wv)
        wo = A_Wo.reshape(HD, D)
        hbm = pl.BlockSpec(memory_space=pltpu.HBM)
        out = pl.pallas_call(
            functools.partial(kernel, bh=bh, bh2=bh2, bw2=bw2, bw3=bw3, bw4=bw4),
            out_shape=jax.ShapeDtypeStruct((S, D), BF16),
            in_specs=[hbm] * 10,
            out_specs=hbm,
            scratch_shapes=[
                pltpu.VMEM((S, D), BF16), pltpu.VMEM((M, D), BF16),
                pltpu.VMEM((HD, D), BF16), pltpu.VMEM((HD, D), BF16), pltpu.VMEM((HD, D), BF16), pltpu.VMEM((HD, D), BF16),
                pltpu.VMEM((D, D), BF16), pltpu.VMEM((D, D), BF16), pltpu.VMEM((D, FF), BF16), pltpu.VMEM((FF, D), BF16),
                pltpu.VMEM(((NSEG + 2) * SEG, D), F32),
                pltpu.VMEM((2, (NSEG + 2) * SEG, D), F32),
                pltpu.VMEM(((NSEG + 2) * SEG, D), BF16),
                pltpu.VMEM((2 * SEG + 2 * M, D), BF16),
                pltpu.SemaphoreType.DMA((10,)),
            ],
            compiler_params=pltpu.CompilerParams(vmem_limit_bytes=110 * 1024 * 1024),
        )(x, mem0, wq, wk, wv, wo, B_w1, B_w2, B_w3, B_w4)
        return out.reshape(1, S, D)
    return fn


_fn = make(bh=1, bh2=2, bw2=3, bw3=15, bw4=100)


@functools.partial(jax.jit, static_argnames=["A_seg_len"])
def pallas_interleave_layers__memory_aug_recurrent_mem_tr__mixer_s_mlp__prompt_kernel(
        A_x, A_mem0, A_Wq, A_Wk, A_Wv, A_Wo, A_seg_len, B_x, B_w1, B_w2, B_w3, B_w4):
    assert A_seg_len == SEG
    return _fn(A_x, A_mem0, A_Wq, A_Wk, A_Wv, A_Wo, A_seg_len, B_x, B_w1, B_w2, B_w3, B_w4)
```

```python
import functools
import numpy as np
import jax
import jax.numpy as jnp
from jax import lax
from jax.experimental import pallas as pl
from jax.experimental.pallas import tpu as pltpu

F32 = jnp.float32
BF16 = jnp.bfloat16

S, D, H, DH, M, SEG, FF = 2048, 640, 32, 192, 8, 32, 1536
NSEG = S // SEG
HD = H * DH
NP = H // 2
PW = 2 * DH
LAG = 3
NT_DIMS = (((1,), (1,)), ((), ()))
SCALE = float(DH) ** -0.5


def _ln(x):
    m = jnp.mean(x, axis=-1, keepdims=True)
    c = x - m
    v = jnp.mean(c * c, axis=-1, keepdims=True)
    return c * lax.rsqrt(v + 1e-5)


def _gelu(x):
    return 0.5 * x * (1.0 + jnp.tanh(0.7978845608028654 * (x + 0.044715 * (x * x * x))))


def _rows(s, n=SEG, off=0):
    if isinstance(s, int):
        return pl.ds(s * SEG + off, n)
    return pl.ds(pl.multiple_of(s * SEG, SEG) + off, n)


def kernel(x_hbm, mem0_hbm, wq_hbm, wk_hbm, wv_hbm, wo_hbm, w1_hbm, w2_hbm, w3_hbm, w4_hbm,
           out_hbm,
           x0, mem0, wq, wk, wv, wo, w1, w2, w3, w4,
           xr, hb, ob, lhs, sems, psems, osem, *, cfg):
    bh, bh2, bw2, bw3, bw4 = cfg['bpos']

    xfirst = 4 * SEG
    c_x0 = pltpu.make_async_copy(x_hbm.at[pl.ds(0, xfirst)], x0.at[pl.ds(0, xfirst)], sems.at[0])
    c_m0 = pltpu.make_async_copy(mem0_hbm, mem0, sems.at[1])
    c_x0.start()
    c_m0.start()
    pair_cps = []
    for p in range(NP):
        sl = pl.ds(p * PW, PW)
        cps = [pltpu.make_async_copy(s.at[sl], d.at[sl], psems.at[p])
               for s, d in ((wq_hbm, wq), (wk_hbm, wk), (wv_hbm, wv), (wo_hbm, wo))]
        for c in cps:
            c.start()
        pair_cps.append(cps)
    c_x1 = pltpu.make_async_copy(x_hbm.at[pl.ds(xfirst, S - xfirst)], x0.at[pl.ds(xfirst, S - xfirst)], sems.at[2])
    c_w = [pltpu.make_async_copy(s, d, sems.at[3 + i]) for i, (s, d) in
           enumerate(((w1_hbm, w1), (w2_hbm, w2), (w3_hbm, w3), (w4_hbm, w4)))]
    for c in c_w:
        c.start()
    c_x1.start()

    zh = jnp.zeros((8, D), F32)
    for l in range(2):
        hb[l, 0:8, :] = zh
        hb[l, 8 + S:16 + S, :] = zh
    c_x0.wait()
    c_m0.wait()
    m0 = mem0[...]
    lhs[2 * SEG:, :] = jnp.concatenate([m0, m0], axis=0)

    def step(t, a1, a2, h_on, r_on, first=False):
        r48 = lax.broadcasted_iota(jnp.int32, (48, 96), 0)
        c96 = lax.broadcasted_iota(jnp.int32, (48, 96), 1)
        hi = c96 >= 48
        j = jnp.where(hi, c96 - 48, c96)
        lo_l = lax.broadcasted_iota(jnp.int32, (48, 128), 1) < 64
        layers = [l for l, on in enumerate((a1, a2)) if on]
        nl = len(layers)

        xs = {}
        if a1:
            xs[0] = x0[_rows(t), :].astype(F32)
            lhs[0:SEG, :] = _ln(xs[0]).astype(BF16)
        if a2:
            xs[1] = xr[_rows(t - LAG), :]
            lhs[SEG:2 * SEG, :] = _ln(xs[1]).astype(BF16)

        def L():
            if nl == 2:
                return lhs[...]
            if layers[0] == 1:
                return lhs[SEG:, :]
            return jnp.concatenate([lhs[0:SEG, :], lhs[2 * SEG:, :]], axis=0)

        def bd(a):
            z = jnp.zeros((48, 128), BF16)
            a0, a1_, a2_ = a[:, 0:128], a[:, 128:256], a[:, 256:384]
            top = jnp.concatenate([a0, jnp.where(lo_l, a1_, z), z], axis=1)
            bot = jnp.concatenate([z, jnp.where(lo_l, z, a1_), a2_], axis=1)
            return jnp.concatenate([top, bot], axis=0)

        def lrows(a, i):
            if nl == 1:
                return a
            return jnp.concatenate([a[SEG * i:SEG * i + SEG], a[2 * SEG:]], axis=0)

        def proj(w, p):
            c0 = p * PW
            return lax.dot_general(L(), w[c0:c0 + PW, :], NT_DIMS, preferred_element_type=F32).astype(BF16)

        def qk(q, k):
            return [lax.dot_general(lrows(q, i), bd(lrows(k, i)), NT_DIMS, preferred_element_type=F32)
                    for i in range(nl)]

        def softmax(sc, l):
            sc = sc * SCALE
            isx = j < 32
            ismem = (j >= 32 + M * l) & (j < 32 + M * l + M)
            allowed = (isx & ((r48 >= 32) | (j <= r48))) | ismem
            fill = jnp.where(isx, -1e9, -jnp.inf).astype(F32)
            sc = jnp.where(allowed, sc, fill)
            m0_ = jnp.max(jnp.where(hi, -jnp.inf, sc), axis=-1, keepdims=True)
            m1_ = jnp.max(jnp.where(hi, sc, -jnp.inf), axis=-1, keepdims=True)
            e = jnp.exp(sc - jnp.where(hi, m1_, m0_))
            d0 = jnp.sum(jnp.where(hi, 0.0, e), axis=-1, keepdims=True)
            d1 = jnp.sum(jnp.where(hi, e, 0.0), axis=-1, keepdims=True)
            return (e * jnp.where(hi, 1.0 / d1, 1.0 / d0)).astype(BF16)

        def pv(prs, v):
            outs = [jnp.dot(prs[i], bd(lrows(v, i)), preferred_element_type=F32) for i in range(nl)]
            if nl == 1:
                return outs[0].astype(BF16)
            return jnp.concatenate([outs[0][0:32], outs[1][0:32], outs[0][32:40], outs[1][40:48]], axis=0).astype(BF16)

        def oproj(o, p):
            return jnp.dot(o, wo[p * PW:(p + 1) * PW, :], preferred_element_type=F32)

        hsegs = [(l, t - 1 - LAG * l) for l in range(2) if h_on[l]]
        rsegs = [(l, t - 2 - LAG * l) for l in range(2) if r_on[l]]
        st = {}

        def B_h():
            if not hsegs:
                return
            xin = jnp.concatenate([xr[_rows(s), :] for _, s in hsegs], axis=0)
            zz = _ln(_ln(xin)).astype(BF16)
            st['h'] = jnp.dot(zz, w1[...], preferred_element_type=F32)

        def B_h2():
            if not hsegs:
                return
            h = _gelu(st['h'])
            for i, (l, s) in enumerate(hsegs):
                hb[l, _rows(s, off=8), :] = h[i * SEG:(i + 1) * SEG]

        def B_w2():
            if not rsegs:
                return
            lane = lax.broadcasted_iota(jnp.int32, (SEG, D), 1)
            parts = []
            for l, s in rsegs:
                win = hb[l, _rows(s, n=SEG + 16), :]
                g0 = win[7:7 + SEG]
                g1 = win[9:9 + SEG]
                g2 = win[6:6 + SEG]
                g3 = win[10:10 + SEG]
                parts.append(jnp.where(lane < 320, jnp.where(lane < 160, g0, g1), jnp.where(lane < 480, g2, g3)))
            hc = jnp.concatenate(parts, axis=0).astype(BF16)
            st['hs'] = jnp.dot(hc, w2[...], preferred_element_type=F32)

        def B_w3():
            if not rsegs:
                return
            xres = jnp.concatenate([xr[_rows(s), :] for _, s in rsegs], axis=0)
            y1 = _ln(xres) + st['hs']
            st['y1x'] = xres + y1
            z1 = _ln(y1).astype(BF16)
            st['h3'] = jnp.dot(z1, w3[...], preferred_element_type=F32)

        def B_w4():
            if not rsegs:
                return
            h3 = _gelu(st['h3']).astype(BF16)
            st['h4'] = jnp.dot(h3, w4[...], preferred_element_type=F32)

        def B_out():
            if not rsegs:
                return
            xnew = st['y1x'] + st['h4']
            for i, (l, s) in enumerate(rsegs):
                if l == 0:
                    xr[_rows(s), :] = xnew[i * SEG:(i + 1) * SEG]
                else:
                    ob[_rows(s), :] = xnew[i * SEG:(i + 1) * SEG].astype(BF16)
                    if cfg['out_overlap']:
                        pltpu.make_async_copy(ob.at[_rows(s)], out_hbm.at[_rows(s)], osem).start()

        chain = ((bh, B_h), (bh2, B_h2), (bw2, B_w2), (bw3, B_w3), (bw4, B_w4))

        def fill_at(key):
            for kk, f in chain:
                if kk == key:
                    f()

        if nl == 0:
            for _, f in chain:
                f()
            B_out()
            return

        def wait_pair(p):
            if first:
                for c in pair_cps[p]:
                    c.wait()

        acc = None
        wait_pair(0)
        q = proj(wq, 0); k = proj(wk, 0); v = proj(wv, 0)
        sc = qk(q, k)
        for p in range(NP):
            fill_at(p)
            if p + 1 < NP:
                wait_pair(p + 1)
                qn = proj(wq, p + 1)
                kn = proj(wk, p + 1)
            prs = [softmax(sc[i], layers[i]) for i in range(nl)]
            o = pv(prs, v)
            if p + 1 < NP:
                v = proj(wv, p + 1)
                sc = qk(qn, kn)
            else:
                fill_at(100)
            r = oproj(o, p)
            acc = r if acc is None else acc + r
        fill_at(101)
        B_out()

        if a1:
            xr[_rows(t), :] = xs[0] + acc[0:SEG]
        if a2:
            i = layers.index(1)
            xr[_rows(t - LAG), :] = xs[1] + acc[i * SEG:(i + 1) * SEG]
        mm = acc[nl * SEG:].astype(BF16)
        if nl == 2:
            lhs[2 * SEG:, :] = mm
        elif layers[0] == 0:
            rr = lax.broadcasted_iota(jnp.int32, (2 * M, D), 0)
            lhs[2 * SEG:, :] = jnp.where(rr >= M, jnp.concatenate([m0, m0], axis=0), mm)
        else:
            lhs[2 * SEG:, :] = mm

    def flags(t):
        a1 = 0 <= t < NSEG
        a2 = 0 <= t - LAG < NSEG
        h_on = tuple(0 <= t - 1 - LAG * l < NSEG for l in range(2))
        r_on = tuple(0 <= t - 2 - LAG * l < NSEG for l in range(2))
        return a1, a2, h_on, r_on

    T0 = LAG + 2
    for t in range(T0):
        step(t, *flags(t), first=(t == 0))
        if t == 0:
            for c in c_w:
                c.wait()
            c_x1.wait()

    def body(t, carry):
        step(t, True, True, (True, True), (True, True))
        return carry

    lax.fori_loop(T0, NSEG, body, 0)
    for t in range(NSEG, NSEG + LAG + 2):
        step(t, *flags(t))
    if cfg['out_overlap']:
        pltpu.make_async_copy(ob, out_hbm, osem).wait()
    else:
        cp = pltpu.make_async_copy(ob, out_hbm, osem)
        cp.start()
        cp.wait()


def make(bpos=(1, 2, 3, 15, 100), out_overlap=True):
    cfg = dict(bpos=tuple(bpos), out_overlap=out_overlap)

    def fn(A_x, A_mem0, A_Wq, A_Wk, A_Wv, A_Wo, A_seg_len, B_x, B_w1, B_w2, B_w3, B_w4):
        x = A_x.reshape(S, D)
        mem0 = A_mem0.reshape(M, D)
        tr = lambda w: jnp.transpose(w, (1, 2, 0)).reshape(HD, D)
        wq, wk, wv = tr(A_Wq), tr(A_Wk), tr(A_Wv)
        wo = A_Wo.reshape(HD, D)
        hbm = pl.BlockSpec(memory_space=pltpu.HBM)
        out = pl.pallas_call(
            functools.partial(kernel, cfg=cfg),
            out_shape=jax.ShapeDtypeStruct((S, D), BF16),
            in_specs=[hbm] * 10,
            out_specs=hbm,
            scratch_shapes=[
                pltpu.VMEM((S, D), BF16), pltpu.VMEM((M, D), BF16),
                pltpu.VMEM((HD, D), BF16), pltpu.VMEM((HD, D), BF16), pltpu.VMEM((HD, D), BF16), pltpu.VMEM((HD, D), BF16),
                pltpu.VMEM((D, D), BF16), pltpu.VMEM((D, D), BF16), pltpu.VMEM((D, FF), BF16), pltpu.VMEM((FF, D), BF16),
                pltpu.VMEM((S, D), F32),
                pltpu.VMEM((2, S + 16, D), F32),
                pltpu.VMEM((S, D), BF16),
                pltpu.VMEM((2 * SEG + 2 * M, D), BF16),
                pltpu.SemaphoreType.DMA((7,)),
                pltpu.SemaphoreType.DMA((NP,)),
                pltpu.SemaphoreType.DMA,
            ],
            compiler_params=pltpu.CompilerParams(vmem_limit_bytes=110 * 1024 * 1024),
        )(x, mem0, wq, wk, wv, wo, B_w1, B_w2, B_w3, B_w4)
        return out.reshape(1, S, D)
    return fn


_fn = make()


@functools.partial(jax.jit, static_argnames=["A_seg_len"])
def pallas_interleave_layers__memory_aug_recurrent_mem_tr__mixer_s_mlp__prompt_kernel(
        A_x, A_mem0, A_Wq, A_Wk, A_Wv, A_Wo, A_seg_len, B_x, B_w1, B_w2, B_w3, B_w4):
    assert A_seg_len == SEG
    return _fn(A_x, A_mem0, A_Wq, A_Wk, A_Wv, A_Wo, A_seg_len, B_x, B_w1, B_w2, B_w3, B_w4)
```

```python
import functools
import numpy as np
import jax
import jax.numpy as jnp
from jax import lax
from jax.experimental import pallas as pl
from jax.experimental.pallas import tpu as pltpu

F32 = jnp.float32
BF16 = jnp.bfloat16

S, D, H, DH, M, SEG, FF = 2048, 640, 32, 192, 8, 32, 1536
NSEG = S // SEG
HD = H * DH
NP = H // 2
PW = 2 * DH
LAG = 3
NT_DIMS = (((1,), (1,)), ((), ()))
NN_DIMS = (((1,), (0,)), ((), ()))
HSEG = 16
SCALE = float(DH) ** -0.5


def _ln(x):
    m = jnp.mean(x, axis=-1, keepdims=True)
    c = x - m
    v = jnp.mean(c * c, axis=-1, keepdims=True)
    return c * lax.rsqrt(v + 1e-5)


def _gelu(x):
    return 0.5 * x * (1.0 + jnp.tanh(0.7978845608028654 * (x + 0.044715 * (x * x * x))))


def _rows(s, n=SEG, off=0):
    if isinstance(s, int):
        return pl.ds(s * SEG + off, n)
    return pl.ds(pl.multiple_of(s * SEG, SEG) + off, n)


def kernel(x_hbm, mem0_hbm, wq_hbm, wk_hbm, wv_hbm, wo_hbm, w1_hbm, w2_hbm, w3_hbm, w4_hbm,
           out_hbm,
           x0, mem0, wq, wk, wv, wo, w1, w2, w3, w4,
           xr, hb, ob, lhs, lhsp, pre, sems, psems, osem, *, cfg):
    bh, bh2, bw2, bw3, bw4 = cfg['bpos']

    NPRE = cfg['npre']
    WIN = cfg['win']
    xfirst = (LAG + NPRE + 1) * SEG
    c_x0 = pltpu.make_async_copy(x_hbm.at[pl.ds(0, xfirst)], x0.at[pl.ds(0, xfirst)], sems.at[0])
    c_m0 = pltpu.make_async_copy(mem0_hbm, mem0, sems.at[1])
    c_x0.start()
    c_m0.start()
    pair_cps = []
    for p in range(NP):
        sl = pl.ds(p * PW, PW)
        pair_cps.append([pltpu.make_async_copy(s.at[sl], d.at[sl], psems.at[p])
                         for s, d in ((wq_hbm, wq), (wk_hbm, wk), (wv_hbm, wv), (wo_hbm, wo))])
    c_x1 = pltpu.make_async_copy(x_hbm.at[pl.ds(xfirst, S - xfirst)], x0.at[pl.ds(xfirst, S - xfirst)], sems.at[2])
    c_w = [pltpu.make_async_copy(s, d, sems.at[3 + i]) for i, (s, d) in
           enumerate(((w1_hbm, w1), (w2_hbm, w2), (w3_hbm, w3), (w4_hbm, w4)))]

    def start_group(p):
        if p < NP:
            for c in pair_cps[p]:
                c.start()
        elif p == NP:
            for c in c_w:
                c.start()
            c_x1.start()

    if cfg.get('dev'):
        for p in range(NP + 1):
            start_group(p)
    else:
        start_group(0)

    zh = jnp.zeros((8, D), F32)
    for l in range(2):
        hb[l, 0:8, :] = zh
        hb[l, 8 + S:16 + S, :] = zh
    with jax.named_scope("sc_wait0"):
        c_x0.wait()
        c_m0.wait()
    if not cfg.get('dev'):
        for p in range(1, WIN):
            start_group(p)
    m0 = mem0[...].astype(F32)
    lhs[2 * SEG:, :] = jnp.concatenate([m0, m0], axis=0).astype(BF16)
    with jax.named_scope("sc_lnp"):
      for i in range(NPRE):
        lhsp[i * HSEG:(i + 1) * HSEG, :] = _ln(x0[_rows(LAG + i, n=HSEG), :].astype(F32)).astype(BF16)

    def step(t, a1, a2, h_on, r_on, first=False, usep=False):
        r40 = lax.broadcasted_iota(jnp.int32, (40, 128), 0)
        c128 = lax.broadcasted_iota(jnp.int32, (40, 128), 1)
        hi = c128 >= 40
        j = jnp.where(hi, c128 - 40, c128)
        in0 = c128 < 40
        in1 = hi & (c128 < 80)
        lo_l = c128 < 64
        layers = [l for l, on in enumerate((a1, a2)) if on]
        nl = len(layers)
        nx = nl * SEG

        xs = {}
        if a1:
            xs[0] = x0[_rows(t), :].astype(F32)
            if usep:
                lhs[HSEG:SEG, :] = _ln(xs[0][HSEG:]).astype(BF16)
            else:
                lhs[0:SEG, :] = _ln(xs[0]).astype(BF16)
        if a2:
            xs[1] = xr[_rows(t - LAG), :]
            lhs[SEG:2 * SEG, :] = _ln(xs[1]).astype(BF16)

        def L():
            if nl == 2:
                return lhs[HSEG:, :] if usep else lhs[...]
            if layers[0] == 1:
                return lhs[SEG:, :]
            return jnp.concatenate([lhs[0:SEG, :], lhs[2 * SEG:, :]], axis=0)

        def bd(a):
            z = jnp.zeros((40, 128), F32)
            a0, a1_, a2_ = a[:, 0:128], a[:, 128:256], a[:, 256:384]
            top = jnp.concatenate([a0, jnp.where(lo_l, a1_, z), z], axis=1)
            bot = jnp.concatenate([z, jnp.where(lo_l, z, a1_), a2_], axis=1)
            return jnp.concatenate([top, bot], axis=0).astype(BF16)

        def lrows(a, i):
            l = layers[i]
            return jnp.concatenate([a[SEG * i:SEG * i + SEG], a[nx + M * l:nx + M * l + M]], axis=0)

        def proj(m, p):
            c0 = p * PW
            w = (wq, wk, wv)[m]
            r = lax.dot_general(L(), w[c0:c0 + PW, :], NT_DIMS, preferred_element_type=F32)
            if usep:
                ps = t - LAG
                prow = pl.ds(ps * HSEG, HSEG) if isinstance(ps, int) else pl.ds(pl.multiple_of(ps * HSEG, HSEG), HSEG)
                r = jnp.concatenate([pre[m, prow, c0:c0 + PW].astype(F32), r], axis=0)
            if first and NPRE:
                pre[m, :, c0:c0 + PW] = lax.dot_general(
                    lhsp[...], w[c0:c0 + PW, :], NT_DIMS, preferred_element_type=F32).astype(BF16)
            return r

        def qk(q, k):
            return [lax.dot_general(lrows(q, i), bd(lrows(k, i)), NT_DIMS, preferred_element_type=F32)
                    for i in range(nl)]

        def softmax(sc):
            sc = jnp.concatenate([sc * SCALE, jnp.zeros((40, 48), F32)], axis=1)
            allowed = (j >= 32) | (r40 >= 32) | (j <= r40)
            sc = jnp.where(allowed, sc, -1e9)
            m0_ = jnp.max(jnp.where(in0, sc, -jnp.inf), axis=-1, keepdims=True)
            m1_ = jnp.max(jnp.where(in1, sc, -jnp.inf), axis=-1, keepdims=True)
            e = jnp.exp(sc - jnp.where(hi, m1_, m0_))
            d0 = jnp.sum(jnp.where(in0, e, 0.0), axis=-1, keepdims=True)
            d1 = jnp.sum(jnp.where(in1, e, 0.0), axis=-1, keepdims=True)
            return (e * jnp.where(hi, 1.0 / d1, 1.0 / d0))[:, 0:80]

        def pv(prs, v):
            outs = [lax.dot_general(prs[i], bd(lrows(v, i)), NN_DIMS, preferred_element_type=F32)
                    for i in range(nl)]
            if nl == 1:
                return outs[0]
            return jnp.concatenate([outs[0][0:32], outs[1][0:32], outs[0][32:40], outs[1][32:40]], axis=0).astype(BF16)

        def oproj(o, p):
            return lax.dot_general(o, wo[p * PW:(p + 1) * PW, :], NN_DIMS, preferred_element_type=F32)

        hsegs = [(l, t - 1 - LAG * l) for l in range(2) if h_on[l]]
        rsegs = [(l, t - 2 - LAG * l) for l in range(2) if r_on[l]]
        st = {}

        def B_h():
            if not hsegs:
                return
            if isinstance(t, int) and t == 1:
                c_w[0].wait()
            xin = jnp.concatenate([xr[_rows(s), :] for _, s in hsegs], axis=0)
            zz = _ln(_ln(xin)).astype(BF16)
            st['h'] = jnp.dot(zz, w1[...], preferred_element_type=F32)

        def B_h2():
            if not hsegs:
                return
            h = _gelu(st['h'])
            for i, (l, s) in enumerate(hsegs):
                hb[l, _rows(s, off=8), :] = h[i * SEG:(i + 1) * SEG]

        def B_w2():
            if not rsegs:
                return
            if isinstance(t, int) and t == 2:
                c_w[1].wait()
                c_w[2].wait()
                c_w[3].wait()
                c_x1.wait()
            lane = lax.broadcasted_iota(jnp.int32, (SEG, D), 1)
            parts = []
            for l, s in rsegs:
                win = hb[l, _rows(s, n=SEG + 16), :]
                g0 = win[7:7 + SEG]
                g1 = win[9:9 + SEG]
                g2 = win[6:6 + SEG]
                g3 = win[10:10 + SEG]
                parts.append(jnp.where(lane < 320, jnp.where(lane < 160, g0, g1), jnp.where(lane < 480, g2, g3)))
            hc = jnp.concatenate(parts, axis=0).astype(BF16)
            st['hs'] = jnp.dot(hc, w2[...], preferred_element_type=F32)

        def B_w3():
            if not rsegs:
                return
            xres = jnp.concatenate([xr[_rows(s), :] for _, s in rsegs], axis=0)
            y1 = _ln(xres) + st['hs']
            st['y1x'] = xres + y1
            z1 = _ln(y1).astype(BF16)
            st['h3'] = jnp.dot(z1, w3[...], preferred_element_type=F32)

        def B_w4():
            if not rsegs:
                return
            h3 = _gelu(st['h3']).astype(BF16)
            st['h4'] = jnp.dot(h3, w4[...], preferred_element_type=F32)

        def B_out():
            if not rsegs:
                return
            xnew = st['y1x'] + st['h4']
            for i, (l, s) in enumerate(rsegs):
                if l == 0:
                    xr[_rows(s), :] = xnew[i * SEG:(i + 1) * SEG]
                else:
                    ob[_rows(s), :] = xnew[i * SEG:(i + 1) * SEG].astype(BF16)
                    if cfg['out_overlap']:
                        pltpu.make_async_copy(ob.at[_rows(s)], out_hbm.at[_rows(s)], osem).start()

        chain = ((bh, B_h), (bh2, B_h2), (bw2, B_w2), (bw3, B_w3), (bw4, B_w4))

        def fill_at(key):
            for kk, f in chain:
                if kk == key:
                    f()

        if nl == 0:
            for _, f in chain:
                f()
            B_out()
            return

        def wait_pair(p):
            if first:
                for c in pair_cps[p]:
                    c.wait()
                start_group(p + WIN)

        acc = None
        wait_pair(0)
        q = proj(0, 0); k = proj(1, 0); v = proj(2, 0)
        sc = qk(q, k)
        for p in range(NP):
            fill_at(p)
            if p + 1 < NP:
                wait_pair(p + 1)
                qn = proj(0, p + 1)
                kn = proj(1, p + 1)
            prs = [softmax(sc[i]) for i in range(nl)]
            o = pv(prs, v)
            if p + 1 < NP:
                v = proj(2, p + 1)
                sc = qk(qn, kn)
            else:
                fill_at(100)
            r = oproj(o, p)
            acc = r if acc is None else acc + r
        fill_at(101)
        B_out()

        if a1:
            xr[_rows(t), :] = xs[0] + acc[0:SEG]
        if a2:
            i = layers.index(1)
            xr[_rows(t - LAG), :] = xs[1] + acc[i * SEG:(i + 1) * SEG]
        if nl == 2:
            lhs[2 * SEG:, :] = acc[nx:].astype(BF16)
        elif layers[0] == 0:
            lhs[2 * SEG:, :] = jnp.concatenate([acc[nx:], m0], axis=0).astype(BF16)
        else:
            lhs[2 * SEG:, :] = jnp.concatenate([m0, acc[nx:]], axis=0).astype(BF16)

    def flags(t):
        a1 = 0 <= t < NSEG
        a2 = 0 <= t - LAG < NSEG
        h_on = tuple(0 <= t - 1 - LAG * l < NSEG for l in range(2))
        r_on = tuple(0 <= t - 2 - LAG * l < NSEG for l in range(2))
        return a1, a2, h_on, r_on

    T0 = LAG + 2
    if cfg.get('dev'):
        for cps in pair_cps:
            for c in cps:
                c.wait()
        for c in c_w:
            c.wait()
        c_x1.wait()
        xr[...] = jnp.zeros(xr.shape, F32)
        hb[...] = jnp.zeros(hb.shape, F32)
    if cfg.get('only0'):
        T0 = 1
    for t in range(0 if cfg.get('dev') else T0):
        with jax.named_scope(f"sc_t{t}"):
            step(t, *flags(t), first=(t == 0), usep=(LAG <= t < LAG + NPRE))
        if t == 0 and cfg.get('only0'):
            for c in c_w:
                c.wait()
            c_x1.wait()

    def body(t, carry, usep):
        step(t, True, True, (True, True), (True, True), usep=usep)
        return carry

    T1 = max(T0, LAG + NPRE)
    if cfg.get('only0'):
        ob[0:SEG, :] = xr[0:SEG, :].astype(BF16)
        cp = pltpu.make_async_copy(ob.at[0:SEG], out_hbm.at[0:SEG], osem)
        cp.start()
        cp.wait()
        return
    if cfg.get('dev'):
        lax.fori_loop(T0, NSEG, functools.partial(body, usep=cfg.get('devp', False)), 0)
    else:
        with jax.named_scope("sc_loopP"):
            if T1 > T0:
                lax.fori_loop(T0, T1, functools.partial(body, usep=True), 0)
        with jax.named_scope("sc_loop"):
            lax.fori_loop(T1, NSEG, functools.partial(body, usep=False), 0)
    for t in range(NSEG, NSEG if cfg.get('dev') else NSEG + LAG + 2):
        with jax.named_scope(f"sc_t{t}"):
            step(t, *flags(t))
    if cfg['out_overlap']:
        pltpu.make_async_copy(ob, out_hbm, osem).wait()
    else:
        cp = pltpu.make_async_copy(ob, out_hbm, osem)
        cp.start()
        cp.wait()


def make(bpos=(1, 2, 3, 15, 100), out_overlap=True, npre=16, win=2, **kw):
    cfg = dict(bpos=tuple(bpos), out_overlap=out_overlap, npre=npre, win=win, **kw)

    def fn(A_x, A_mem0, A_Wq, A_Wk, A_Wv, A_Wo, A_seg_len, B_x, B_w1, B_w2, B_w3, B_w4):
        x = A_x.reshape(S, D)
        mem0 = A_mem0.reshape(M, D)
        tr = lambda w: jnp.transpose(w, (1, 2, 0)).reshape(HD, D)
        wq, wk, wv = tr(A_Wq), tr(A_Wk), tr(A_Wv)
        wo = A_Wo.reshape(HD, D)
        hbm = pl.BlockSpec(memory_space=pltpu.HBM)
        out = pl.pallas_call(
            functools.partial(kernel, cfg=cfg),
            out_shape=jax.ShapeDtypeStruct((S, D), BF16),
            in_specs=[hbm] * 10,
            out_specs=hbm,
            scratch_shapes=[
                pltpu.VMEM((S, D), BF16), pltpu.VMEM((M, D), BF16),
                pltpu.VMEM((HD, D), BF16), pltpu.VMEM((HD, D), BF16), pltpu.VMEM((HD, D), BF16), pltpu.VMEM((HD, D), BF16),
                pltpu.VMEM((D, D), BF16), pltpu.VMEM((D, D), BF16), pltpu.VMEM((D, FF), BF16), pltpu.VMEM((FF, D), BF16),
                pltpu.VMEM((S, D), F32),
                pltpu.VMEM((2, S + 16, D), F32),
                pltpu.VMEM((S, D), BF16),
                pltpu.VMEM((2 * SEG + 2 * M, D), BF16),
                pltpu.VMEM((cfg['npre'] * HSEG, D), BF16),
                pltpu.VMEM((3, cfg['npre'] * HSEG, HD), BF16),
                pltpu.SemaphoreType.DMA((7,)),
                pltpu.SemaphoreType.DMA((NP,)),
                pltpu.SemaphoreType.DMA,
            ],
            compiler_params=pltpu.CompilerParams(vmem_limit_bytes=110 * 1024 * 1024),
        )(x, mem0, wq, wk, wv, wo, B_w1, B_w2, B_w3, B_w4)
        return out.reshape(1, S, D)
    return fn


_fn = make(npre=15)


@functools.partial(jax.jit, static_argnames=["A_seg_len"])
def pallas_interleave_layers__memory_aug_recurrent_mem_tr__mixer_s_mlp__prompt_kernel(
        A_x, A_mem0, A_Wq, A_Wk, A_Wv, A_Wo, A_seg_len, B_x, B_w1, B_w2, B_w3, B_w4):
    assert A_seg_len == SEG
    return _fn(A_x, A_mem0, A_Wq, A_Wk, A_Wv, A_Wo, A_seg_len, B_x, B_w1, B_w2, B_w3, B_w4)
```

```python
import functools
import numpy as np
import jax
import jax.numpy as jnp
from jax import lax
from jax.experimental import pallas as pl
from jax.experimental.pallas import tpu as pltpu

F32 = jnp.float32
BF16 = jnp.bfloat16

S, D, H, DH, M, SEG, FF = 2048, 640, 32, 192, 8, 32, 1536
NSEG = S // SEG
HD = H * DH
NP = H // 2
PW = 2 * DH
LAG = 3
NT_DIMS = (((1,), (1,)), ((), ()))
NN_DIMS = (((1,), (0,)), ((), ()))
HSEG = 16
SCALE = float(DH) ** -0.5


def _ln(x):
    m = jnp.mean(x, axis=-1, keepdims=True)
    c = x - m
    v = jnp.mean(c * c, axis=-1, keepdims=True)
    return c * lax.rsqrt(v + 1e-5)


def _gelu(x):
    return 0.5 * x * (1.0 + jnp.tanh(0.7978845608028654 * (x + 0.044715 * (x * x * x))))


def _rows(s, n=SEG, off=0):
    if isinstance(s, int):
        return pl.ds(s * SEG + off, n)
    return pl.ds(pl.multiple_of(s * SEG, SEG) + off, n)


def kernel(x_hbm, mem0_hbm, wq_hbm, wk_hbm, wv_hbm, wo_hbm, w1_hbm, w2_hbm, w3_hbm, w4_hbm,
           out_hbm,
           x0, mem0, wq, wk, wv, wo, w1, w2, w3, w4,
           xr, hb, ob, lhs, lhsp, pre, wn, wop, sems, psems, osem, *, cfg):
    bh, bh2, bw2, bw3, bw4 = cfg['bpos']

    NPRE = cfg['npre']
    WIN = cfg['win']
    xfirst = (LAG + NPRE + 1) * SEG
    c_x0 = pltpu.make_async_copy(x_hbm.at[pl.ds(0, xfirst)], x0.at[pl.ds(0, xfirst)], sems.at[0])
    c_m0 = pltpu.make_async_copy(mem0_hbm, mem0, sems.at[1])
    c_x0.start()
    c_m0.start()
    pair_cps = []
    for p in range(NP):
        sl = pl.ds(p * PW, PW)
        pair_cps.append([pltpu.make_async_copy(s.at[sl], d.at[sl], psems.at[p])
                         for s, d in ((wq_hbm, wq), (wk_hbm, wk), (wv_hbm, wv), (wo_hbm, wo))])
    c_x1 = pltpu.make_async_copy(x_hbm.at[pl.ds(xfirst, S - xfirst)], x0.at[pl.ds(xfirst, S - xfirst)], sems.at[2])
    c_w = [pltpu.make_async_copy(s, d, sems.at[3 + i]) for i, (s, d) in
           enumerate(((w1_hbm, w1), (w2_hbm, w2), (w3_hbm, w3), (w4_hbm, w4)))]

    def start_group(p):
        if p < NP:
            for c in pair_cps[p]:
                c.start()
        elif p == NP:
            for c in c_w:
                c.start()
            c_x1.start()

    if cfg.get('dev'):
        for p in range(NP + 1):
            start_group(p)
    else:
        start_group(0)

    zh = jnp.zeros((8, D), F32)
    for l in range(2):
        hb[l, 0:8, :] = zh
        hb[l, 8 + S:16 + S, :] = zh
    with jax.named_scope("sc_wait0"):
        c_x0.wait()
        c_m0.wait()
    if not cfg.get('dev'):
        for p in range(1, WIN):
            start_group(p)
    m0 = mem0[...].astype(F32)
    lhs[2 * SEG:, :] = jnp.concatenate([m0, m0], axis=0).astype(BF16)
    with jax.named_scope("sc_lnp"):
      for i in range(NPRE):
        lhsp[i * HSEG:(i + 1) * HSEG, :] = _ln(x0[_rows(LAG + i, n=HSEG), :].astype(F32)).astype(BF16)

    def step(t, a1, a2, h_on, r_on, first=False, usep=False):
        r40 = lax.broadcasted_iota(jnp.int32, (40, 128), 0)
        c128 = lax.broadcasted_iota(jnp.int32, (40, 128), 1)
        hi = c128 >= 40
        j = jnp.where(hi, c128 - 40, c128)
        in0 = c128 < 40
        in1 = hi & (c128 < 80)
        lo_l = c128 < 64
        layers = [l for l, on in enumerate((a1, a2)) if on]
        nl = len(layers)
        nx = nl * SEG

        xs = {}
        if a1:
            xs[0] = x0[_rows(t), :].astype(F32)
            if usep:
                lhs[HSEG:SEG, :] = _ln(xs[0][HSEG:]).astype(BF16)
            else:
                lhs[0:SEG, :] = _ln(xs[0]).astype(BF16)
        if a2:
            xs[1] = xr[_rows(t - LAG), :]
            lhs[SEG:2 * SEG, :] = _ln(xs[1]).astype(BF16)

        def L():
            if nl == 2:
                return lhs[HSEG:, :] if usep else lhs[...]
            if layers[0] == 1:
                return lhs[SEG:, :]
            return jnp.concatenate([lhs[0:SEG, :], lhs[2 * SEG:, :]], axis=0)

        def bd(a):
            z = jnp.zeros((40, 128), F32)
            a0, a1_, a2_ = a[:, 0:128], a[:, 128:256], a[:, 256:384]
            top = jnp.concatenate([a0, jnp.where(lo_l, a1_, z), z], axis=1)
            bot = jnp.concatenate([z, jnp.where(lo_l, z, a1_), a2_], axis=1)
            return jnp.concatenate([top, bot], axis=0).astype(BF16)

        def lrows(a, i):
            l = layers[i]
            return jnp.concatenate([a[SEG * i:SEG * i + SEG], a[nx + M * l:nx + M * l + M]], axis=0)

        def proj(m, p):
            c0 = p * PW
            if first or not cfg.get('nn', True):
                w = (wq, wk, wv)[m][c0:c0 + PW, :]
                r = lax.dot_general(L(), w, NT_DIMS, preferred_element_type=F32)
                if first and NPRE:
                    pre[m, :, c0:c0 + PW] = lax.dot_general(
                        lhsp[...], w, NT_DIMS, preferred_element_type=F32).astype(BF16)
                if first and cfg.get('nn', True):
                    wn[m, :, c0:c0 + PW] = pltpu.bitcast(w.T, jnp.uint32)
            else:
                w = pltpu.bitcast(wn[m, :, c0:c0 + PW], BF16)
                r = lax.dot_general(L(), w, NN_DIMS, preferred_element_type=F32)
            if usep:
                ps = t - LAG
                prow = pl.ds(ps * HSEG, HSEG) if isinstance(ps, int) else pl.ds(pl.multiple_of(ps * HSEG, HSEG), HSEG)
                r = jnp.concatenate([pre[m, prow, c0:c0 + PW].astype(F32), r], axis=0)
            return r

        def qk(q, k):
            return [lax.dot_general(lrows(q, i), bd(lrows(k, i)), NT_DIMS, preferred_element_type=F32)
                    for i in range(nl)]

        def softmax(sc):
            sc = jnp.concatenate([sc * SCALE, jnp.zeros((40, 48), F32)], axis=1)
            allowed = (j >= 32) | (r40 >= 32) | (j <= r40)
            sc = jnp.where(allowed, sc, -1e9)
            m0_ = jnp.max(jnp.where(in0, sc, -jnp.inf), axis=-1, keepdims=True)
            m1_ = jnp.max(jnp.where(in1, sc, -jnp.inf), axis=-1, keepdims=True)
            e = jnp.exp(sc - jnp.where(hi, m1_, m0_))
            d0 = jnp.sum(jnp.where(in0, e, 0.0), axis=-1, keepdims=True)
            d1 = jnp.sum(jnp.where(in1, e, 0.0), axis=-1, keepdims=True)
            return (e * jnp.where(hi, 1.0 / d1, 1.0 / d0))[:, 0:80]

        def pv(prs, v):
            outs = [lax.dot_general(prs[i], bd(lrows(v, i)), NN_DIMS, preferred_element_type=F32)
                    for i in range(nl)]
            if nl == 1:
                return outs[0]
            return jnp.concatenate([outs[0][0:32], outs[1][0:32], outs[0][32:40], outs[1][32:40]], axis=0).astype(BF16)

        def oproj(o, p):
            if first or not cfg.get('wop', True):
                w = wo[p * PW:(p + 1) * PW, :]
                if first and cfg.get('wop', True):
                    wop[p * PW // 2:(p + 1) * PW // 2, :] = pltpu.bitcast(w, jnp.uint32)
            else:
                w = pltpu.bitcast(wop[p * PW // 2:(p + 1) * PW // 2, :], BF16)
            return lax.dot_general(o, w, NN_DIMS, preferred_element_type=F32)

        hsegs = [(l, t - 1 - LAG * l) for l in range(2) if h_on[l]]
        rsegs = [(l, t - 2 - LAG * l) for l in range(2) if r_on[l]]
        st = {}

        def B_h():
            if not hsegs:
                return
            if isinstance(t, int) and t == 1:
                c_w[0].wait()
            xin = jnp.concatenate([xr[_rows(s), :] for _, s in hsegs], axis=0)
            zz = _ln(_ln(xin)).astype(BF16)
            st['h'] = jnp.dot(zz, w1[...], preferred_element_type=F32)

        def B_h2():
            if not hsegs:
                return
            h = _gelu(st['h'])
            for i, (l, s) in enumerate(hsegs):
                hb[l, _rows(s, off=8), :] = h[i * SEG:(i + 1) * SEG]

        def B_w2():
            if not rsegs:
                return
            if isinstance(t, int) and t == 2:
                c_w[1].wait()
                c_w[2].wait()
                c_w[3].wait()
                c_x1.wait()
            lane = lax.broadcasted_iota(jnp.int32, (SEG, D), 1)
            parts = []
            for l, s in rsegs:
                win = hb[l, _rows(s, n=SEG + 16), :]
                g0 = win[7:7 + SEG]
                g1 = win[9:9 + SEG]
                g2 = win[6:6 + SEG]
                g3 = win[10:10 + SEG]
                parts.append(jnp.where(lane < 320, jnp.where(lane < 160, g0, g1), jnp.where(lane < 480, g2, g3)))
            hc = jnp.concatenate(parts, axis=0).astype(BF16)
            st['hs'] = jnp.dot(hc, w2[...], preferred_element_type=F32)

        def B_w3():
            if not rsegs:
                return
            xres = jnp.concatenate([xr[_rows(s), :] for _, s in rsegs], axis=0)
            y1 = _ln(xres) + st['hs']
            st['y1x'] = xres + y1
            z1 = _ln(y1).astype(BF16)
            st['h3'] = jnp.dot(z1, w3[...], preferred_element_type=F32)

        def B_w4():
            if not rsegs:
                return
            h3 = _gelu(st['h3']).astype(BF16)
            st['h4'] = jnp.dot(h3, w4[...], preferred_element_type=F32)

        def B_out():
            if not rsegs:
                return
            xnew = st['y1x'] + st['h4']
            for i, (l, s) in enumerate(rsegs):
                if l == 0:
                    xr[_rows(s), :] = xnew[i * SEG:(i + 1) * SEG]
                else:
                    ob[_rows(s), :] = xnew[i * SEG:(i + 1) * SEG].astype(BF16)
                    if cfg['out_overlap']:
                        pltpu.make_async_copy(ob.at[_rows(s)], out_hbm.at[_rows(s)], osem).start()

        chain = ((bh, B_h), (bh2, B_h2), (bw2, B_w2), (bw3, B_w3), (bw4, B_w4))

        def fill_at(key):
            for kk, f in chain:
                if kk == key:
                    f()

        if nl == 0:
            for _, f in chain:
                f()
            B_out()
            return

        def wait_pair(p):
            if first:
                for c in pair_cps[p]:
                    c.wait()
                start_group(p + WIN)

        acc = None
        wait_pair(0)
        q = proj(0, 0); k = proj(1, 0); v = proj(2, 0)
        sc = qk(q, k)
        for p in range(NP):
            fill_at(p)
            if p + 1 < NP:
                wait_pair(p + 1)
                qn = proj(0, p + 1)
                kn = proj(1, p + 1)
            prs = [softmax(sc[i]) for i in range(nl)]
            o = pv(prs, v)
            if p + 1 < NP:
                v = proj(2, p + 1)
                sc = qk(qn, kn)
            else:
                fill_at(100)
            r = oproj(o, p)
            acc = r if acc is None else acc + r
        fill_at(101)
        B_out()

        if a1:
            xr[_rows(t), :] = xs[0] + acc[0:SEG]
        if a2:
            i = layers.index(1)
            xr[_rows(t - LAG), :] = xs[1] + acc[i * SEG:(i + 1) * SEG]
        if nl == 2:
            lhs[2 * SEG:, :] = acc[nx:].astype(BF16)
        elif layers[0] == 0:
            lhs[2 * SEG:, :] = jnp.concatenate([acc[nx:], m0], axis=0).astype(BF16)
        else:
            lhs[2 * SEG:, :] = jnp.concatenate([m0, acc[nx:]], axis=0).astype(BF16)

    def flags(t):
        a1 = 0 <= t < NSEG
        a2 = 0 <= t - LAG < NSEG
        h_on = tuple(0 <= t - 1 - LAG * l < NSEG for l in range(2))
        r_on = tuple(0 <= t - 2 - LAG * l < NSEG for l in range(2))
        return a1, a2, h_on, r_on

    T0 = LAG + 2
    if cfg.get('dev'):
        for cps in pair_cps:
            for c in cps:
                c.wait()
        for c in c_w:
            c.wait()
        c_x1.wait()
        xr[...] = jnp.zeros(xr.shape, F32)
        hb[...] = jnp.zeros(hb.shape, F32)
    if cfg.get('only0'):
        T0 = 1
    for t in range(0 if cfg.get('dev') else T0):
        with jax.named_scope(f"sc_t{t}"):
            step(t, *flags(t), first=(t == 0), usep=(LAG <= t < LAG + NPRE))
        if t == 0 and cfg.get('only0'):
            for c in c_w:
                c.wait()
            c_x1.wait()

    def body(t, carry, usep):
        step(t, True, True, (True, True), (True, True), usep=usep)
        return carry

    T1 = max(T0, LAG + NPRE)
    if cfg.get('only0'):
        ob[0:SEG, :] = xr[0:SEG, :].astype(BF16)
        cp = pltpu.make_async_copy(ob.at[0:SEG], out_hbm.at[0:SEG], osem)
        cp.start()
        cp.wait()
        return
    if cfg.get('dev'):
        lax.fori_loop(T0, NSEG, functools.partial(body, usep=cfg.get('devp', False)), 0)
    else:
        with jax.named_scope("sc_loopP"):
            if T1 > T0:
                lax.fori_loop(T0, T1, functools.partial(body, usep=True), 0)
        with jax.named_scope("sc_loop"):
            lax.fori_loop(T1, NSEG, functools.partial(body, usep=False), 0)
    for t in range(NSEG, NSEG if cfg.get('dev') else NSEG + LAG + 2):
        with jax.named_scope(f"sc_t{t}"):
            step(t, *flags(t))
    if cfg['out_overlap']:
        pltpu.make_async_copy(ob, out_hbm, osem).wait()
    else:
        cp = pltpu.make_async_copy(ob, out_hbm, osem)
        cp.start()
        cp.wait()


def make(bpos=(1, 2, 3, 15, 100), out_overlap=True, npre=16, win=2, **kw):
    cfg = dict(bpos=tuple(bpos), out_overlap=out_overlap, npre=npre, win=win, **kw)

    def fn(A_x, A_mem0, A_Wq, A_Wk, A_Wv, A_Wo, A_seg_len, B_x, B_w1, B_w2, B_w3, B_w4):
        x = A_x.reshape(S, D)
        mem0 = A_mem0.reshape(M, D)
        tr = lambda w: jnp.transpose(w, (1, 2, 0)).reshape(HD, D)
        wq, wk, wv = tr(A_Wq), tr(A_Wk), tr(A_Wv)
        wo = A_Wo.reshape(HD, D)
        hbm = pl.BlockSpec(memory_space=pltpu.HBM)
        out = pl.pallas_call(
            functools.partial(kernel, cfg=cfg),
            out_shape=jax.ShapeDtypeStruct((S, D), BF16),
            in_specs=[hbm] * 10,
            out_specs=hbm,
            scratch_shapes=[
                pltpu.VMEM((S, D), BF16), pltpu.VMEM((M, D), BF16),
                pltpu.VMEM((HD, D), BF16), pltpu.VMEM((HD, D), BF16), pltpu.VMEM((HD, D), BF16), pltpu.VMEM((HD, D), BF16),
                pltpu.VMEM((D, D), BF16), pltpu.VMEM((D, D), BF16), pltpu.VMEM((D, FF), BF16), pltpu.VMEM((FF, D), BF16),
                pltpu.VMEM((S, D), F32),
                pltpu.VMEM((2, S + 16, D), F32),
                pltpu.VMEM((S, D), BF16),
                pltpu.VMEM((2 * SEG + 2 * M, D), BF16),
                pltpu.VMEM((max(cfg['npre'], 1) * HSEG, D), BF16),
                pltpu.VMEM((3, max(cfg['npre'], 1) * HSEG, HD), BF16),
                pltpu.VMEM((3, D // 2, HD), jnp.uint32),
                pltpu.VMEM((HD // 2, D), jnp.uint32),
                pltpu.SemaphoreType.DMA((7,)),
                pltpu.SemaphoreType.DMA((NP,)),
                pltpu.SemaphoreType.DMA,
            ],
            compiler_params=pltpu.CompilerParams(vmem_limit_bytes=110 * 1024 * 1024),
        )(x, mem0, wq, wk, wv, wo, B_w1, B_w2, B_w3, B_w4)
        return out.reshape(1, S, D)
    return fn


_fn = make(npre=15)


@functools.partial(jax.jit, static_argnames=["A_seg_len"])
def pallas_interleave_layers__memory_aug_recurrent_mem_tr__mixer_s_mlp__prompt_kernel(
        A_x, A_mem0, A_Wq, A_Wk, A_Wv, A_Wo, A_seg_len, B_x, B_w1, B_w2, B_w3, B_w4):
    assert A_seg_len == SEG
    return _fn(A_x, A_mem0, A_Wq, A_Wk, A_Wv, A_Wo, A_seg_len, B_x, B_w1, B_w2, B_w3, B_w4)
```

```python
import functools
import numpy as np
import jax
import jax.numpy as jnp
from jax import lax
from jax.experimental import pallas as pl
from jax.experimental.pallas import tpu as pltpu

F32 = jnp.float32
BF16 = jnp.bfloat16
U32 = jnp.uint32

S, D, H, DH, M, SEG, FF = 2048, 640, 32, 192, 8, 32, 1536
NSEG = S // SEG
HD = H * DH
NP = H // 2
PW = 2 * DH
LAG = 3
NT_DIMS = (((1,), (1,)), ((), ()))
NN_DIMS = (((1,), (0,)), ((), ()))
HSEG = 16
SCALE = float(DH) ** -0.5


def _ln(x):
    m = jnp.mean(x, axis=-1, keepdims=True)
    c = x - m
    v = jnp.mean(c * c, axis=-1, keepdims=True)
    return c * lax.rsqrt(v + 1e-5)


def _gelu(x):
    return 0.5 * x * (1.0 + jnp.tanh(0.7978845608028654 * (x + 0.044715 * (x * x * x))))


def _rows(s, n=SEG, off=0):
    if isinstance(s, int):
        return pl.ds(s * SEG + off, n)
    return pl.ds(pl.multiple_of(s * SEG, SEG) + off, n)


def _slot(s, n=SEG, off=0):
    if isinstance(s, int):
        return pl.ds((min(max(s, -1), NSEG) + 1) * SEG + off, n)
    return pl.ds(pl.multiple_of((jnp.clip(s, -1, NSEG) + 1) * SEG, SEG) + off, n)


def _valid(s):
    return (s >= 0) & (s < NSEG)


def kernel(x_hbm, mem0_hbm, wq_hbm, wk_hbm, wv_hbm, wo_hbm, w1_hbm, w2_hbm, w3_hbm, w4_hbm,
           out_hbm,
           x0, mem0, wq, wk, wv, wo, w1, w2, w3, w4,
           xr, hb, ob, lhs, lhsp, pre, wn, lhsf, memf, sems, psems, osem, *, cfg):
    bh, bh2, bw2, bw3, bw4 = cfg['bpos']

    NPRE = cfg['npre']
    WIN = cfg['win']
    xfirst = (LAG + NPRE + 1) * SEG
    c_x0 = pltpu.make_async_copy(x_hbm.at[pl.ds(0, xfirst)], x0.at[pl.ds(0, xfirst)], sems.at[0])
    c_m0 = pltpu.make_async_copy(mem0_hbm, mem0, sems.at[1])
    c_x0.start()
    c_m0.start()
    mats = ((wq_hbm, wq), (wk_hbm, wk), (wv_hbm, wv), (wo_hbm, wo))
    PW2 = PW // 2

    def prow(p):
        if isinstance(p, int):
            return pl.ds(p * PW2, PW2)
        return pl.ds(pl.multiple_of(p * PW2, 8), PW2)

    def group(p):
        return [pltpu.make_async_copy(s_.bitcast(U32).at[prow(p)], d_.at[prow(p)], psems.at[p]) for s_, d_ in mats]

    c_x1 = pltpu.make_async_copy(x_hbm.at[pl.ds(xfirst, S - xfirst)], x0.at[pl.ds(xfirst, S - xfirst)], sems.at[2])
    c_w = [pltpu.make_async_copy(s.bitcast(U32), d, sems.at[3 + i]) for i, (s, d) in
           enumerate(((w1_hbm, w1), (w2_hbm, w2), (w3_hbm, w3), (w4_hbm, w4)))]

    def start_group(p):
        if p < NP:
            for c in group(p):
                c.start()
        elif p == NP:
            for c in c_w:
                c.start()
            c_x1.start()

    if cfg.get('dev'):
        for p in range(NP + 1):
            start_group(p)
    else:
        start_group(0)

    zh = jnp.zeros((SEG, D), F32)
    for l in range(2):
        hb[l, _slot(-1), :] = zh
        hb[l, _slot(NSEG), :] = zh
        hb[l, _slot(0), :] = zh
        hb[l, _slot(1), :] = zh
    xr[_slot(-1), :] = zh
    xr[_slot(NSEG), :] = zh
    with jax.named_scope("sc_wait0"):
        c_x0.wait()
        c_m0.wait()
    if not cfg.get('dev'):
        for p in range(1, WIN):
            start_group(p)
    m0 = mem0[...].astype(F32)
    m00 = jnp.concatenate([m0, m0], axis=0)
    NPR = NPRE * HSEG
    with jax.named_scope("sc_lnp"):
        for i in range(NPRE):
            lhsp[i * HSEG:(i + 1) * HSEG, :] = _ln(x0[_rows(LAG + i, n=HSEG), :].astype(F32)).astype(BF16)
        lhsp[NPR + SEG:, :] = m00.astype(BF16)
        memf[...] = m00
        lhs[2 * SEG:, :] = m00.astype(BF16)

    def ub(x):
        return pltpu.bitcast(x, BF16)

    def bu(x):
        return pltpu.bitcast(x, U32)

    def step(t, a1, a2, h_on, r_on, first=False, usep=False, dummy=False, waitw=False, last=False):
        r40 = lax.broadcasted_iota(jnp.int32, (40, 128), 0)
        c128 = lax.broadcasted_iota(jnp.int32, (40, 128), 1)
        hi = c128 >= 40
        j = jnp.where(hi, c128 - 40, c128)
        in0 = c128 < 40
        in1 = hi & (c128 < 80)
        lo_l = c128 < 64
        layers = [l for l, on in enumerate((a1, a2)) if on]
        nl = len(layers)
        nx = nl * SEG

        xs = {}
        f32l = nl == 1 and not first
        if a1:
            xs[0] = x0[_rows(t), :].astype(F32)
            if first:
                lhsp[NPR:NPR + SEG, :] = _ln(xs[0]).astype(BF16)
            elif f32l:
                lhsf[0:SEG, :] = _ln(xs[0])
            elif usep:
                lhs[HSEG:SEG, :] = _ln(xs[0][HSEG:]).astype(BF16)
            else:
                lhs[0:SEG, :] = _ln(xs[0]).astype(BF16)
        if a2:
            xs[1] = xr[_slot(t - LAG), :]
            if f32l:
                lhsf[0:SEG, :] = _ln(xs[1])
            else:
                lhs[SEG:2 * SEG, :] = _ln(xs[1]).astype(BF16)
        if f32l:
            lhsf[SEG:, :] = memf[M * layers[0]:M * layers[0] + M, :]

        def L():
            if first:
                return lhsp[...]
            if nl == 2:
                return lhs[HSEG:, :] if usep else lhs[...]
            return lhsf[...]

        def bd(a):
            z = jnp.zeros((40, 128), F32)
            a0, a1_, a2_ = a[:, 0:128], a[:, 128:256], a[:, 256:384]
            top = jnp.concatenate([a0, jnp.where(lo_l, a1_, z), z], axis=1)
            bot = jnp.concatenate([z, jnp.where(lo_l, z, a1_), a2_], axis=1)
            return jnp.concatenate([top, bot], axis=0).astype(BF16)

        def lrows(a, i):
            if nl == 1:
                return a[0:SEG + M]
            l = layers[i]
            return jnp.concatenate([a[SEG * i:SEG * i + SEG], a[nx + M * l:nx + M * l + M]], axis=0)

        def proj(m, p):
            if first:
                w = ub((wq, wk, wv)[m][prow(p), :])
                r = lax.dot_general(L(), w, NT_DIMS, preferred_element_type=F32)
                wn[m, p] = bu(w.T)
                if NPRE:
                    pre[m, p] = bu(r[0:NPR].astype(BF16))
                return r[NPR:]
            w = ub(wn[m, p])
            r = lax.dot_general(L(), w, NN_DIMS, preferred_element_type=F32)
            if usep:
                ps = t - LAG
                h2 = HSEG // 2
                pr_ = pl.ds(ps * h2, h2) if isinstance(ps, int) else pl.ds(pl.multiple_of(ps * h2, h2), h2)
                r = jnp.concatenate([ub(pre[m, p, pr_, :]).astype(F32), r], axis=0)
            return r

        def qk(q, k):
            return [lax.dot_general(lrows(q, i), bd(lrows(k, i)), NT_DIMS, preferred_element_type=F32)
                    for i in range(nl)]

        def softmax(sc):
            sc = jnp.concatenate([sc * SCALE, jnp.zeros((40, 48), F32)], axis=1)
            allowed = ((j >= 32) | (r40 >= 32) | (j <= r40)) & (c128 < 80)
            sc = jnp.where(allowed, sc, -1e9)
            m0_ = jnp.max(jnp.where(in0, sc, -jnp.inf), axis=-1, keepdims=True)
            m1_ = jnp.max(jnp.where(in1, sc, -jnp.inf), axis=-1, keepdims=True)
            e = jnp.exp(sc - jnp.where(hi, m1_, m0_))
            d0 = jnp.sum(jnp.where(in0, e, 0.0), axis=-1, keepdims=True)
            d1 = jnp.sum(jnp.where(in1, e, 0.0), axis=-1, keepdims=True)
            return (e * jnp.where(hi, 1.0 / d1, 1.0 / d0))[:, 0:80]

        def pv(prs, v):
            outs = [lax.dot_general(prs[i], bd(lrows(v, i)), NN_DIMS, preferred_element_type=F32)
                    for i in range(nl)]
            if nl == 1:
                return outs[0]
            return jnp.concatenate([outs[0][0:32], outs[1][0:32], outs[0][32:40], outs[1][32:40]], axis=0).astype(BF16)

        def oproj(o, p):
            w = ub(wo[prow(p), :])
            return lax.dot_general(o, w, NN_DIMS, preferred_element_type=F32)

        hsegs = [(l, t - 1 - LAG * l) for l in range(2) if h_on[l]]
        rsegs = [(l, t - 2 - LAG * l) for l in range(2) if r_on[l]]
        if last:
            rsegs = [(1, NSEG - 2), (1, NSEG - 1)]
        st = {}

        def B_h():
            if not hsegs:
                return
            xin = jnp.concatenate([xr[_slot(s), :] for _, s in hsegs], axis=0)
            zz = _ln(_ln(xin)).astype(BF16)
            st['h'] = jnp.dot(zz, ub(w1[...]), preferred_element_type=F32)

        def B_h2():
            if not hsegs:
                return
            h = _gelu(st['h'])
            for i, (l, s) in enumerate(hsegs):
                hv = h[i * SEG:(i + 1) * SEG]
                if dummy:
                    hv = jnp.where(_valid(s), hv, 0.0)
                hb[l, _slot(s), :] = hv

        def B_w2():
            if not rsegs:
                return
            if waitw:
                @pl.when(t == 1)
                def _():
                    c_w[1].wait()
                    c_w[2].wait()
                    c_w[3].wait()
            lane = lax.broadcasted_iota(jnp.int32, (SEG, D), 1)
            parts = []
            for l, s in rsegs:
                sc_ = jnp.clip(s, 0, NSEG - 1) if dummy else s
                win = hb[l, _slot(sc_, n=SEG + 16, off=-8), :]
                g0 = win[7:7 + SEG]
                g1 = win[9:9 + SEG]
                g2 = win[6:6 + SEG]
                g3 = win[10:10 + SEG]
                parts.append(jnp.where(lane < 320, jnp.where(lane < 160, g0, g1), jnp.where(lane < 480, g2, g3)))
            hc = jnp.concatenate(parts, axis=0).astype(BF16)
            st['hs'] = jnp.dot(hc, ub(w2[...]), preferred_element_type=F32)

        def B_w3():
            if not rsegs:
                return
            xres = jnp.concatenate([xr[_slot(s), :] for _, s in rsegs], axis=0)
            y1 = _ln(xres) + st['hs']
            st['y1x'] = xres + y1
            z1 = _ln(y1).astype(BF16)
            st['h3'] = jnp.dot(z1, ub(w3[...]), preferred_element_type=F32)

        def B_w4():
            if not rsegs:
                return
            h3 = _gelu(st['h3']).astype(BF16)
            st['h4'] = jnp.dot(h3, ub(w4[...]), preferred_element_type=F32)

        def B_out():
            if not rsegs:
                return
            xnew = st['y1x'] + st['h4']
            for i, (l, s) in enumerate(rsegs):
                if l == 0:
                    xr[_slot(s), :] = xnew[i * SEG:(i + 1) * SEG]
                else:
                    ob[_slot(s), :] = xnew[i * SEG:(i + 1) * SEG].astype(BF16)
                    st.setdefault('out', []).append(s)

        chain = ((bh, B_h), (bh2, B_h2), (bw2, B_w2), (bw3, B_w3), (bw4, B_w4))

        def fill_at(key):
            for kk, f in chain:
                if kk == key:
                    f()

        def send_out():
            if 'out' not in st:
                return
            for s_ in st['out']:
                def go(s_=s_):
                    pltpu.make_async_copy(ob.at[_slot(s_)], out_hbm.at[_rows(s_)], osem).start()

                if dummy:
                    pl.when(s_ >= 0)(go)
                else:
                    go()

        if nl == 0:
            for _, f in chain:
                f()
            B_out()
            send_out()
            return

        if first:
            def pair_body(p, carry):
                sc_prev, v_prev, acc = carry
                for c in group(p):
                    c.wait()

                @pl.when(p + WIN < NP)
                def _():
                    for c in group(p + WIN):
                        c.start()

                @pl.when(p == cfg.get('bstart', NP - 1))
                def _():
                    start_group(NP)

                q = proj(0, p)
                k = proj(1, p)
                o = pv([softmax(sc_prev)], v_prev)
                v = proj(2, p)
                sc = qk(q, k)
                acc = acc + oproj(o, jnp.maximum(p - 1, 0))
                return sc[0], v[0:SEG + M], acc

            init = (jnp.zeros((SEG + M, 80), F32), jnp.zeros((SEG + M, PW), F32), jnp.zeros((SEG + M, D), F32))
            sc_l, v_l, acc = lax.fori_loop(0, NP, pair_body, init)
            acc = acc + oproj(pv([softmax(sc_l)], v_l), NP - 1)
        else:
            acc = None
            q = proj(0, 0); k = proj(1, 0); v = proj(2, 0)
            sc = qk(q, k)
            for p in range(NP):
                fill_at(p)
                if p + 1 < NP:
                    qn = proj(0, p + 1)
                    kn = proj(1, p + 1)
                prs = [softmax(sc[i]) for i in range(nl)]
                o = pv(prs, v)
                if p + 1 < NP:
                    v = proj(2, p + 1)
                    sc = qk(qn, kn)
                else:
                    fill_at(100)
                r = oproj(o, p)
                acc = r if acc is None else acc + r
            fill_at(101)
            B_out()

        if a1:
            xr[_slot(t), :] = xs[0] + acc[0:SEG]
        if a2:
            i = layers.index(1)
            xr[_slot(t - LAG), :] = xs[1] + acc[i * SEG:(i + 1) * SEG]
        if nl == 2:
            mm = acc[nx:]
        elif layers[0] == 0:
            mm = jnp.concatenate([acc[nx:], m0], axis=0)
        else:
            mm = jnp.concatenate([m0, acc[nx:]], axis=0)
        memf[...] = mm
        lhs[2 * SEG:, :] = mm.astype(BF16)
        send_out()

    def flags(t):
        a1 = 0 <= t < NSEG
        a2 = 0 <= t - LAG < NSEG
        h_on = tuple(0 <= t - 1 - LAG * l < NSEG for l in range(2))
        r_on = tuple(0 <= t - 2 - LAG * l < NSEG for l in range(2))
        return a1, a2, h_on, r_on

    def scope(name):
        return jax.named_scope(name)

    with scope("sc_t0"):
        step(0, *flags(0), first=True)
    ON, OFF = True, False

    def loop(name, lo, hi, *fl, **kw):
        with scope(name):
            lax.fori_loop(lo, hi, lambda t, c: (step(t, *fl, **kw), c)[1], 0)

    mode = cfg.get('mode', 'loops')
    if mode == 'loops':
        if cfg.get('head', 'loop') == 'loop':
            for c in c_w:
                c.wait()
            loop("sc_head", 1, LAG, ON, OFF, (ON, OFF), (ON, OFF), dummy=True)
        elif cfg['head'] == 'loopw':
            c_w[0].wait()
            loop("sc_head", 1, LAG, ON, OFF, (ON, OFF), (ON, OFF), dummy=True, waitw=True)
        else:
            for t in range(1, LAG):
                if t == 1:
                    c_w[0].wait()
                if t == 2:
                    c_w[1].wait()
                    c_w[2].wait()
                    c_w[3].wait()
                with scope(f"sc_t{t}"):
                    step(t, *flags(t))
        T1 = max(LAG, LAG + NPRE)
        loop("sc_loopP", LAG, T1, ON, ON, (ON, ON), (ON, ON), usep=True, dummy=True)
        c_x1.wait()
        loop("sc_loop", T1, NSEG, ON, ON, (ON, ON), (ON, ON))
        if cfg.get('tail', 'loop') == 'loop':
            loop("sc_tail", NSEG, NSEG + LAG, OFF, ON, (ON, ON), (ON, ON), dummy=True)
        else:
            for t in range(NSEG, NSEG + LAG):
                with scope(f"sc_t{t}"):
                    step(t, *flags(t))
    if cfg.get('mergelast', True):
        with scope("sc_last"):
            step(NSEG + LAG, *flags(NSEG + LAG), last=True)
    else:
        for t in range(NSEG + LAG, NSEG + LAG + 2):
            with scope(f"sc_t{t}"):
                step(t, *flags(t))
    pltpu.make_async_copy(ob.at[pl.ds(SEG, S)], out_hbm, osem).wait()


def make(bpos=(1, 2, 3, 15, 100), out_overlap=True, npre=16, win=2, **kw):
    cfg = dict(bpos=tuple(bpos), out_overlap=out_overlap, npre=npre, win=win, **kw)

    def fn(A_x, A_mem0, A_Wq, A_Wk, A_Wv, A_Wo, A_seg_len, B_x, B_w1, B_w2, B_w3, B_w4):
        x = A_x.reshape(S, D)
        mem0 = A_mem0.reshape(M, D)
        tr = lambda w: jnp.transpose(w, (1, 2, 0)).reshape(HD, D)
        wq, wk, wv = tr(A_Wq), tr(A_Wk), tr(A_Wv)
        wo = A_Wo.reshape(HD, D)
        hbm = pl.BlockSpec(memory_space=pltpu.HBM)
        out = pl.pallas_call(
            functools.partial(kernel, cfg=cfg),
            out_shape=jax.ShapeDtypeStruct((S, D), BF16),
            in_specs=[hbm] * 10,
            out_specs=hbm,
            scratch_shapes=[
                pltpu.VMEM((S, D), BF16), pltpu.VMEM((M, D), BF16),
                pltpu.VMEM((HD // 2, D), U32), pltpu.VMEM((HD // 2, D), U32), pltpu.VMEM((HD // 2, D), U32),
                pltpu.VMEM((HD // 2, D), U32),
                pltpu.VMEM((D // 2, D), U32), pltpu.VMEM((D // 2, D), U32),
                pltpu.VMEM((D // 2, FF), U32), pltpu.VMEM((FF // 2, D), U32),
                pltpu.VMEM((S + 2 * SEG, D), F32),
                pltpu.VMEM((2, S + 2 * SEG, D), F32),
                pltpu.VMEM((S + 2 * SEG, D), BF16),
                pltpu.VMEM((2 * SEG + 2 * M, D), BF16),
                pltpu.VMEM((cfg['npre'] * HSEG + SEG + 2 * M, D), BF16),
                pltpu.VMEM((3, NP, max(cfg['npre'], 1) * HSEG // 2, PW), U32),
                pltpu.VMEM((3, NP, D // 2, PW), U32),
                pltpu.VMEM((SEG + M, D), F32),
                pltpu.VMEM((2 * M, D), F32),
                pltpu.SemaphoreType.DMA((7,)),
                pltpu.SemaphoreType.DMA((NP,)),
                pltpu.SemaphoreType.DMA,
            ],
            compiler_params=pltpu.CompilerParams(vmem_limit_bytes=110 * 1024 * 1024),
        )(x, mem0, wq, wk, wv, wo, B_w1, B_w2, B_w3, B_w4)
        return out.reshape(1, S, D)
    return fn


_fn = make(npre=15, head="unroll", tail="unroll")


@functools.partial(jax.jit, static_argnames=["A_seg_len"])
def pallas_interleave_layers__memory_aug_recurrent_mem_tr__mixer_s_mlp__prompt_kernel(
        A_x, A_mem0, A_Wq, A_Wk, A_Wv, A_Wo, A_seg_len, B_x, B_w1, B_w2, B_w3, B_w4):
    assert A_seg_len == SEG
    return _fn(A_x, A_mem0, A_Wq, A_Wk, A_Wv, A_Wo, A_seg_len, B_x, B_w1, B_w2, B_w3, B_w4)
```

```python
import functools
import numpy as np
import jax
import jax.numpy as jnp
from jax import lax
from jax.experimental import pallas as pl
from jax.experimental.pallas import tpu as pltpu

F32 = jnp.float32
BF16 = jnp.bfloat16
U32 = jnp.uint32

S, D, H, DH, M, SEG, FF = 2048, 640, 32, 192, 8, 32, 1536
NSEG = S // SEG
HD = H * DH
NP = H // 2
PW = 2 * DH
LAG = 3
NT_DIMS = (((1,), (1,)), ((), ()))
NN_DIMS = (((1,), (0,)), ((), ()))
HSEG = 16
SCALE = float(DH) ** -0.5


def _ln(x):
    m = jnp.mean(x, axis=-1, keepdims=True)
    c = x - m
    v = jnp.mean(c * c, axis=-1, keepdims=True)
    return c * lax.rsqrt(v + 1e-5)


def _gelu(x):
    return 0.5 * x * (1.0 + jnp.tanh(0.7978845608028654 * (x + 0.044715 * (x * x * x))))


def _rows(s, n=SEG, off=0):
    if isinstance(s, int):
        return pl.ds(s * SEG + off, n)
    return pl.ds(pl.multiple_of(s * SEG, SEG) + off, n)


def _slot(s, n=SEG, off=0):
    if isinstance(s, int):
        return pl.ds((min(max(s, -1), NSEG) + 1) * SEG + off, n)
    return pl.ds(pl.multiple_of((jnp.clip(s, -1, NSEG) + 1) * SEG, SEG) + off, n)


def _valid(s):
    return (s >= 0) & (s < NSEG)


def kernel(x_hbm, mem0_hbm, wq_hbm, wk_hbm, wv_hbm, wo_hbm, w1_hbm, w2_hbm, w3_hbm, w4_hbm,
           out_hbm,
           x0, mem0, wq, wk, wv, wo, w1, w2, w3, w4,
           xr, hb, ob, lhs, lhsp, pre, wn, lhsf, memf, sems, psems, osem, *, cfg):
    bh, bh2, bw2, bw3, bw4 = cfg['bpos']

    NPRE = cfg['npre']
    WIN = cfg['win']
    xfirst = (LAG + NPRE + 1) * SEG
    c_x0 = pltpu.make_async_copy(x_hbm.at[pl.ds(0, xfirst)], x0.at[pl.ds(0, xfirst)], sems.at[0])
    c_m0 = pltpu.make_async_copy(mem0_hbm, mem0, sems.at[1])
    c_x0.start()
    c_m0.start()
    mats = ((wq_hbm, wq), (wk_hbm, wk), (wv_hbm, wv), (wo_hbm, wo))
    PW2 = PW // 2

    def prow(p):
        if isinstance(p, int):
            return pl.ds(p * PW2, PW2)
        return pl.ds(pl.multiple_of(p * PW2, 8), PW2)

    def group(p):
        return [pltpu.make_async_copy(s_.bitcast(U32).at[prow(p)], d_.at[prow(p)], psems.at[p]) for s_, d_ in mats]

    c_x1 = pltpu.make_async_copy(x_hbm.at[pl.ds(xfirst, S - xfirst)], x0.at[pl.ds(xfirst, S - xfirst)], sems.at[2])
    c_w = [pltpu.make_async_copy(s.bitcast(U32), d, sems.at[3 + i]) for i, (s, d) in
           enumerate(((w1_hbm, w1), (w2_hbm, w2), (w3_hbm, w3), (w4_hbm, w4)))]

    def start_group(p):
        if p < NP:
            for c in group(p):
                c.start()
        elif p == NP:
            for c in c_w:
                c.start()
            c_x1.start()

    if cfg.get('dev'):
        for p in range(NP + 1):
            start_group(p)
    else:
        start_group(0)

    zh = jnp.zeros((SEG, D), F32)
    for l in range(2):
        hb[l, _slot(-1), :] = zh
        hb[l, _slot(NSEG), :] = zh
        hb[l, _slot(0), :] = zh
        hb[l, _slot(1), :] = zh
    xr[_slot(-1), :] = zh
    xr[_slot(NSEG), :] = zh
    with jax.named_scope("sc_wait0"):
        c_x0.wait()
        c_m0.wait()
    if not cfg.get('dev'):
        for p in range(1, WIN):
            start_group(p)
    m0 = mem0[...].astype(F32)
    m00 = jnp.concatenate([m0, m0], axis=0)
    NPR = NPRE * HSEG
    with jax.named_scope("sc_lnp"):
        for i in range(NPRE):
            lhsp[i * HSEG:(i + 1) * HSEG, :] = _ln(x0[_rows(LAG + i, n=HSEG), :].astype(F32)).astype(BF16)
        lhsp[NPR + SEG:, :] = m00.astype(BF16)
        memf[...] = m00
        lhs[2 * SEG:, :] = m00.astype(BF16)

    def ub(x):
        return pltpu.bitcast(x, BF16)

    def bu(x):
        return pltpu.bitcast(x, U32)

    def step(t, a1, a2, h_on, r_on, first=False, usep=False, dummy=False, waitw=False, last=False, prepared=False, prep=False):
        r40 = lax.broadcasted_iota(jnp.int32, (40, 128), 0)
        c128 = lax.broadcasted_iota(jnp.int32, (40, 128), 1)
        hi = c128 >= 40
        j = jnp.where(hi, c128 - 40, c128)
        in0 = c128 < 40
        in1 = hi & (c128 < 80)
        lo_l = c128 < 64
        layers = [l for l, on in enumerate((a1, a2)) if on]
        nl = len(layers)
        nx = nl * SEG

        xs = {}
        f32l = nl == 1 and not first
        if a1:
            xs[0] = x0[_rows(t), :].astype(F32)
            if prepared:
                pass
            elif first:
                lhsp[NPR:NPR + SEG, :] = _ln(xs[0]).astype(BF16)
            elif f32l:
                lhsf[0:SEG, :] = _ln(xs[0])
            elif usep:
                lhs[HSEG:SEG, :] = _ln(xs[0][HSEG:]).astype(BF16)
            else:
                lhs[0:SEG, :] = _ln(xs[0]).astype(BF16)
        if a2:
            xs[1] = xr[_slot(t - LAG), :]
            if prepared:
                pass
            elif f32l:
                lhsf[0:SEG, :] = _ln(xs[1])
            else:
                lhs[SEG:2 * SEG, :] = _ln(xs[1]).astype(BF16)
        if f32l:
            lhsf[SEG:, :] = memf[M * layers[0]:M * layers[0] + M, :]

        def L():
            if first:
                return lhsp[...]
            if nl == 2:
                return lhs[HSEG:, :] if usep else lhs[...]
            return lhsf[...]

        def bd(a):
            z = jnp.zeros((40, 128), F32)
            a0, a1_, a2_ = a[:, 0:128], a[:, 128:256], a[:, 256:384]
            top = jnp.concatenate([a0, jnp.where(lo_l, a1_, z), z], axis=1)
            bot = jnp.concatenate([z, jnp.where(lo_l, z, a1_), a2_], axis=1)
            return jnp.concatenate([top, bot], axis=0).astype(BF16)

        def lrows(a, i):
            if nl == 1:
                return a[0:SEG + M]
            l = layers[i]
            return jnp.concatenate([a[SEG * i:SEG * i + SEG], a[nx + M * l:nx + M * l + M]], axis=0)

        def proj(m, p):
            if first:
                w = ub((wq, wk, wv)[m][prow(p), :])
                r = lax.dot_general(L(), w, NT_DIMS, preferred_element_type=F32)
                wn[m, p] = bu(w.T)
                if NPRE:
                    pre[m, p] = bu(r[0:NPR].astype(BF16))
                return r[NPR:]
            w = ub(wn[m, p])
            r = lax.dot_general(L(), w, NN_DIMS, preferred_element_type=F32)
            if usep:
                ps = t - LAG
                h2 = HSEG // 2
                pr_ = pl.ds(ps * h2, h2) if isinstance(ps, int) else pl.ds(pl.multiple_of(ps * h2, h2), h2)
                r = jnp.concatenate([ub(pre[m, p, pr_, :]).astype(F32), r], axis=0)
            return r

        def qk(q, k):
            return [lax.dot_general(lrows(q, i), bd(lrows(k, i)), NT_DIMS, preferred_element_type=F32)
                    for i in range(nl)]

        def softmax(sc):
            sc = jnp.concatenate([sc * SCALE, jnp.zeros((40, 48), F32)], axis=1)
            allowed = ((j >= 32) | (r40 >= 32) | (j <= r40)) & (c128 < 80)
            sc = jnp.where(allowed, sc, -1e9)
            m0_ = jnp.max(jnp.where(in0, sc, -jnp.inf), axis=-1, keepdims=True)
            m1_ = jnp.max(jnp.where(in1, sc, -jnp.inf), axis=-1, keepdims=True)
            e = jnp.exp(sc - jnp.where(hi, m1_, m0_))
            d0 = jnp.sum(jnp.where(in0, e, 0.0), axis=-1, keepdims=True)
            d1 = jnp.sum(jnp.where(in1, e, 0.0), axis=-1, keepdims=True)
            return (e * jnp.where(hi, 1.0 / d1, 1.0 / d0))[:, 0:80]

        def pv(prs, v):
            outs = [lax.dot_general(prs[i], bd(lrows(v, i)), NN_DIMS, preferred_element_type=F32)
                    for i in range(nl)]
            if nl == 1:
                return outs[0]
            return jnp.concatenate([outs[0][0:32], outs[1][0:32], outs[0][32:40], outs[1][32:40]], axis=0).astype(BF16)

        def oproj(o, p):
            w = ub(wo[prow(p), :])
            return lax.dot_general(o, w, NN_DIMS, preferred_element_type=F32)

        hsegs = [(l, t - 1 - LAG * l) for l in range(2) if h_on[l]]
        rsegs = [(l, t - 2 - LAG * l) for l in range(2) if r_on[l]]
        if last:
            rsegs = [(1, NSEG - 2), (1, NSEG - 1)]
        st = {}

        def B_h():
            if not hsegs:
                return
            xin = jnp.concatenate([xr[_slot(s), :] for _, s in hsegs], axis=0)
            zz = _ln(_ln(xin)).astype(BF16)
            st['h'] = jnp.dot(zz, ub(w1[...]), preferred_element_type=F32)

        def B_h2():
            if not hsegs:
                return
            h = _gelu(st['h'])
            for i, (l, s) in enumerate(hsegs):
                hv = h[i * SEG:(i + 1) * SEG]
                if dummy:
                    hv = jnp.where(_valid(s), hv, 0.0)
                hb[l, _slot(s), :] = hv

        def B_w2():
            if not rsegs:
                return
            if waitw:
                @pl.when(t == 1)
                def _():
                    c_w[1].wait()
                    c_w[2].wait()
                    c_w[3].wait()
            lane = lax.broadcasted_iota(jnp.int32, (SEG, D), 1)
            parts = []
            for l, s in rsegs:
                sc_ = jnp.clip(s, 0, NSEG - 1) if dummy else s
                win = hb[l, _slot(sc_, n=SEG + 16, off=-8), :]
                g0 = win[7:7 + SEG]
                g1 = win[9:9 + SEG]
                g2 = win[6:6 + SEG]
                g3 = win[10:10 + SEG]
                parts.append(jnp.where(lane < 320, jnp.where(lane < 160, g0, g1), jnp.where(lane < 480, g2, g3)))
            hc = jnp.concatenate(parts, axis=0).astype(BF16)
            st['hs'] = jnp.dot(hc, ub(w2[...]), preferred_element_type=F32)

        def B_w3():
            if not rsegs:
                return
            xres = jnp.concatenate([xr[_slot(s), :] for _, s in rsegs], axis=0)
            y1 = _ln(xres) + st['hs']
            st['y1x'] = xres + y1
            z1 = _ln(y1).astype(BF16)
            st['h3'] = jnp.dot(z1, ub(w3[...]), preferred_element_type=F32)

        def B_w4():
            if not rsegs:
                return
            h3 = _gelu(st['h3']).astype(BF16)
            ks = cfg.get('w4k', FF)
            if nl == 0:
                ks = FF
            st['h4'] = jnp.dot(h3[:, :ks], ub(w4[0:ks // 2, :]), preferred_element_type=F32)
            st['h3b'] = h3[:, ks:] if ks < FF else None

        def B_w4b():
            if not rsegs or st.get('h3b') is None:
                return
            ks = cfg['w4k']
            st['h4'] = st['h4'] + jnp.dot(st['h3b'], ub(w4[ks // 2:, :]), preferred_element_type=F32)

        def B_out():
            if not rsegs:
                return
            xnew = st['y1x'] + st['h4']
            st['xnew'] = xnew
            for i, (l, s) in enumerate(rsegs):
                if l == 0:
                    xr[_slot(s), :] = xnew[i * SEG:(i + 1) * SEG]
                else:
                    ob[_slot(s), :] = xnew[i * SEG:(i + 1) * SEG].astype(BF16)
                    st.setdefault('out', []).append(s)

        chain = ((bh, B_h), (bh2, B_h2), (bw2, B_w2), (bw3, B_w3), (bw4, B_w4))

        def fill_at(key):
            for kk, f in chain:
                if kk == key:
                    f()

        def send_out():
            if 'out' not in st:
                return
            for s_ in st['out']:
                def go(s_=s_):
                    pltpu.make_async_copy(ob.at[_slot(s_)], out_hbm.at[_rows(s_)], osem).start()

                if dummy:
                    pl.when(s_ >= 0)(go)
                else:
                    go()

        if nl == 0:
            for _, f in chain:
                f()
            B_out()
            send_out()
            return

        if first:
            def pair_body(p, carry):
                sc_prev, v_prev, acc = carry
                for c in group(p):
                    c.wait()

                @pl.when(p + WIN < NP)
                def _():
                    for c in group(p + WIN):
                        c.start()

                @pl.when(p == cfg.get('bstart', NP - 1))
                def _():
                    start_group(NP)

                q = proj(0, p)
                k = proj(1, p)
                o = pv([softmax(sc_prev)], v_prev)
                v = proj(2, p)
                sc = qk(q, k)
                acc = acc + oproj(o, jnp.maximum(p - 1, 0))
                return sc[0], v[0:SEG + M], acc

            init = (jnp.zeros((SEG + M, 80), F32), jnp.zeros((SEG + M, PW), F32), jnp.zeros((SEG + M, D), F32))
            sc_l, v_l, acc = lax.fori_loop(0, NP, pair_body, init)
            acc = acc + oproj(pv([softmax(sc_l)], v_l), NP - 1)
        else:
            acc = None
            q = proj(0, 0); k = proj(1, 0); v = proj(2, 0)
            sc = qk(q, k)
            for p in range(NP):
                fill_at(p)
                if p + 1 < NP:
                    qn = proj(0, p + 1)
                    kn = proj(1, p + 1)
                prs = [softmax(sc[i]) for i in range(nl)]
                o = pv(prs, v)
                if p + 1 < NP:
                    v = proj(2, p + 1)
                    sc = qk(qn, kn)
                else:
                    fill_at(100)
                r = oproj(o, p)
                acc = r if acc is None else acc + r
            fill_at(101)
            B_w4b()
            B_out()

        if a1:
            xr[_slot(t), :] = xs[0] + acc[0:SEG]
        if a2:
            i = layers.index(1)
            xr[_slot(t - LAG), :] = xs[1] + acc[i * SEG:(i + 1) * SEG]
        if nl == 2:
            mm = acc[nx:]
        elif layers[0] == 0:
            mm = jnp.concatenate([acc[nx:], m0], axis=0)
        else:
            mm = jnp.concatenate([m0, acc[nx:]], axis=0)
        if prep:
            tn = min(t + 1, NSEG - 1) if isinstance(t, int) else jnp.minimum(t + 1, NSEG - 1)
            x1n = _ln(x0[_rows(tn), :].astype(F32)).astype(BF16)
            x2n = _ln(st['xnew'][0:SEG]).astype(BF16)
            lhs[0:SEG, :] = x1n
            lhs[SEG:2 * SEG, :] = x2n
        memf[...] = mm
        lhs[2 * SEG:, :] = mm.astype(BF16)
        send_out()

    def flags(t):
        a1 = 0 <= t < NSEG
        a2 = 0 <= t - LAG < NSEG
        h_on = tuple(0 <= t - 1 - LAG * l < NSEG for l in range(2))
        r_on = tuple(0 <= t - 2 - LAG * l < NSEG for l in range(2))
        return a1, a2, h_on, r_on

    def scope(name):
        return jax.named_scope(name)

    PREP = cfg.get('prep', True)
    if cfg.get('bench'):
        for p in range(1 if not cfg.get('dev') else NP + 1, NP + 1):
            if p >= WIN:
                start_group(p)
        for p in range(NP):
            for c in group(p):
                c.wait()
        for c in c_w:
            c.wait()
        c_x1.wait()
        wn[...] = jnp.zeros(wn.shape, U32)
        xr[...] = jnp.zeros(xr.shape, F32)
        hb[...] = jnp.zeros(hb.shape, F32)
        lax.fori_loop(18, NSEG, lambda t, c: (step(t, True, True, (True, True), (True, True), prepared=PREP, prep=PREP), c)[1], 0)
        cp = pltpu.make_async_copy(ob.at[pl.ds(SEG, 46 * SEG)], out_hbm.at[pl.ds(0, 46 * SEG)], osem)
        cp.wait()
        return
    with scope("sc_t0"):
        step(0, *flags(0), first=True)
    ON, OFF = True, False

    def loop(name, lo, hi, *fl, **kw):
        with scope(name):
            lax.fori_loop(lo, hi, lambda t, c: (step(t, *fl, **kw), c)[1], 0)

    mode = cfg.get('mode', 'loops')
    if mode == 'loops':
        if cfg.get('head', 'loop') == 'loop':
            for c in c_w:
                c.wait()
            loop("sc_head", 1, LAG, ON, OFF, (ON, OFF), (ON, OFF), dummy=True)
        elif cfg['head'] == 'loopw':
            c_w[0].wait()
            loop("sc_head", 1, LAG, ON, OFF, (ON, OFF), (ON, OFF), dummy=True, waitw=True)
        else:
            for t in range(1, LAG):
                if t == 1:
                    c_w[0].wait()
                if t == 2:
                    c_w[1].wait()
                    c_w[2].wait()
                    c_w[3].wait()
                with scope(f"sc_t{t}"):
                    step(t, *flags(t), prep=(PREP and t == LAG - 1))
        T1 = max(LAG, LAG + NPRE)
        loop("sc_loopP", LAG, T1, ON, ON, (ON, ON), (ON, ON), usep=True, dummy=True, prepared=PREP, prep=PREP)
        c_x1.wait()
        loop("sc_loop", T1, NSEG, ON, ON, (ON, ON), (ON, ON), prepared=PREP, prep=PREP)
        if cfg.get('tail', 'loop') == 'loop':
            loop("sc_tail", NSEG, NSEG + LAG, OFF, ON, (ON, ON), (ON, ON), dummy=True)
        else:
            for t in range(NSEG, NSEG + LAG):
                with scope(f"sc_t{t}"):
                    step(t, *flags(t))
    if cfg.get('mergelast', True):
        with scope("sc_last"):
            step(NSEG + LAG, *flags(NSEG + LAG), last=True)
    else:
        for t in range(NSEG + LAG, NSEG + LAG + 2):
            with scope(f"sc_t{t}"):
                step(t, *flags(t))
    pltpu.make_async_copy(ob.at[pl.ds(SEG, S)], out_hbm, osem).wait()


def make(bpos=(1, 2, 3, 15, 100), out_overlap=True, npre=16, win=2, **kw):
    cfg = dict(bpos=tuple(bpos), out_overlap=out_overlap, npre=npre, win=win, **kw)

    def fn(A_x, A_mem0, A_Wq, A_Wk, A_Wv, A_Wo, A_seg_len, B_x, B_w1, B_w2, B_w3, B_w4):
        x = A_x.reshape(S, D)
        mem0 = A_mem0.reshape(M, D)
        tr = lambda w: jnp.transpose(w, (1, 2, 0)).reshape(HD, D)
        wq, wk, wv = tr(A_Wq), tr(A_Wk), tr(A_Wv)
        wo = A_Wo.reshape(HD, D)
        hbm = pl.BlockSpec(memory_space=pltpu.HBM)
        out = pl.pallas_call(
            functools.partial(kernel, cfg=cfg),
            out_shape=jax.ShapeDtypeStruct((S, D), BF16),
            in_specs=[hbm] * 10,
            out_specs=hbm,
            scratch_shapes=[
                pltpu.VMEM((S, D), BF16), pltpu.VMEM((M, D), BF16),
                pltpu.VMEM((HD // 2, D), U32), pltpu.VMEM((HD // 2, D), U32), pltpu.VMEM((HD // 2, D), U32),
                pltpu.VMEM((HD // 2, D), U32),
                pltpu.VMEM((D // 2, D), U32), pltpu.VMEM((D // 2, D), U32),
                pltpu.VMEM((D // 2, FF), U32), pltpu.VMEM((FF // 2, D), U32),
                pltpu.VMEM((S + 2 * SEG, D), F32),
                pltpu.VMEM((2, S + 2 * SEG, D), F32),
                pltpu.VMEM((S + 2 * SEG, D), BF16),
                pltpu.VMEM((2 * SEG + 2 * M, D), BF16),
                pltpu.VMEM((cfg['npre'] * HSEG + SEG + 2 * M, D), BF16),
                pltpu.VMEM((3, NP, max(cfg['npre'], 1) * HSEG // 2, PW), U32),
                pltpu.VMEM((3, NP, D // 2, PW), U32),
                pltpu.VMEM((SEG + M, D), F32),
                pltpu.VMEM((2 * M, D), F32),
                pltpu.SemaphoreType.DMA((7,)),
                pltpu.SemaphoreType.DMA((NP,)),
                pltpu.SemaphoreType.DMA,
            ],
            compiler_params=pltpu.CompilerParams(vmem_limit_bytes=110 * 1024 * 1024),
        )(x, mem0, wq, wk, wv, wo, B_w1, B_w2, B_w3, B_w4)
        return out.reshape(1, S, D)
    return fn


_fn = make(npre=15, head="unroll", tail="unroll")


@functools.partial(jax.jit, static_argnames=["A_seg_len"])
def pallas_interleave_layers__memory_aug_recurrent_mem_tr__mixer_s_mlp__prompt_kernel(
        A_x, A_mem0, A_Wq, A_Wk, A_Wv, A_Wo, A_seg_len, B_x, B_w1, B_w2, B_w3, B_w4):
    assert A_seg_len == SEG
    return _fn(A_x, A_mem0, A_Wq, A_Wk, A_Wv, A_Wo, A_seg_len, B_x, B_w1, B_w2, B_w3, B_w4)
```

```python
import functools
import numpy as np
import jax
import jax.numpy as jnp
from jax import lax
from jax.experimental import pallas as pl
from jax.experimental.pallas import tpu as pltpu

F32 = jnp.float32
BF16 = jnp.bfloat16
U32 = jnp.uint32

S, D, H, DH, M, SEG, FF = 2048, 640, 32, 192, 8, 32, 1536
NSEG = S // SEG
HD = H * DH
NP = H // 2
PW = 2 * DH
LAG = 3
NT_DIMS = (((1,), (1,)), ((), ()))
NN_DIMS = (((1,), (0,)), ((), ()))
HSEG = 16
SCALE = float(DH) ** -0.5


def _ln(x):
    m = jnp.mean(x, axis=-1, keepdims=True)
    c = x - m
    v = jnp.mean(c * c, axis=-1, keepdims=True)
    return c * lax.rsqrt(v + 1e-5)


def _gelu(x):
    return 0.5 * x * (1.0 + jnp.tanh(0.7978845608028654 * (x + 0.044715 * (x * x * x))))


def _rows(s, n=SEG, off=0):
    if isinstance(s, int):
        return pl.ds(s * SEG + off, n)
    return pl.ds(pl.multiple_of(s * SEG, SEG) + off, n)


def _slot(s, n=SEG, off=0):
    if isinstance(s, int):
        return pl.ds((min(max(s, -1), NSEG) + 1) * SEG + off, n)
    return pl.ds(pl.multiple_of((jnp.clip(s, -1, NSEG) + 1) * SEG, SEG) + off, n)


def ub(x):
    return pltpu.bitcast(x, BF16)


def bu(x):
    return pltpu.bitcast(x, U32)


def _half(sl):
    st = sl.start
    st = st // 2 if isinstance(st, int) else pl.multiple_of(lax.shift_right_logical(st, 1), 8)
    return pl.ds(st, sl.size // 2)


def _valid(s):
    return (s >= 0) & (s < NSEG)


def kernel(x_hbm, mem0_hbm, wq_hbm, wk_hbm, wv_hbm, wo_hbm, w1_hbm, w2_hbm, w3_hbm, w4_hbm,
           out_hbm,
           x0, mem0, wq, wk, wv, wo, w1, w2, w3, w4,
           xr, hb, ob, lhs, lhsp, pre, wn, lhsf, sems, psems, osem, *, cfg):
    bh, bh2, bw2, bw3, bw4 = cfg['bpos']

    out_u = out_hbm.bitcast(U32)
    NPRE = cfg['npre']
    WIN = cfg['win']
    xfirst = (LAG + NPRE + 1) * SEG
    xu = x_hbm.bitcast(U32)
    c_x0 = pltpu.make_async_copy(xu.at[pl.ds(0, xfirst // 2)], x0.at[pl.ds(0, xfirst // 2)], sems.at[0])
    c_m0 = pltpu.make_async_copy(mem0_hbm, mem0, sems.at[1])
    c_x0.start()
    c_m0.start()
    mats = ((wq_hbm, wq), (wk_hbm, wk), (wv_hbm, wv), (wo_hbm, wo))
    PW2 = PW // 2

    def prow(p):
        if isinstance(p, int):
            return pl.ds(p * PW2, PW2)
        return pl.ds(pl.multiple_of(p * PW2, 8), PW2)

    def group(p):
        return [pltpu.make_async_copy(s_.bitcast(U32).at[prow(p)], d_.at[prow(p)], psems.at[p]) for s_, d_ in mats]

    c_x1 = pltpu.make_async_copy(xu.at[pl.ds(xfirst // 2, (S - xfirst) // 2)],
                                 x0.at[pl.ds(xfirst // 2, (S - xfirst) // 2)], sems.at[2])
    c_w = [pltpu.make_async_copy(s.bitcast(U32), d, sems.at[3 + i]) for i, (s, d) in
           enumerate(((w1_hbm, w1), (w2_hbm, w2), (w3_hbm, w3), (w4_hbm, w4)))]

    def start_group(p):
        if p < NP:
            for c in group(p):
                c.start()
        elif p == NP:
            for c in c_w:
                c.start()
            c_x1.start()

    if cfg.get('dev'):
        for p in range(NP + 1):
            start_group(p)
    else:
        start_group(0)

    zh = jnp.zeros((SEG, D), F32)
    for l in range(2):
        hb[l, _slot(-1), :] = zh
        hb[l, _slot(NSEG), :] = zh
        hb[l, _slot(0), :] = zh
        hb[l, _slot(1), :] = zh
    xr[_slot(-1), :] = zh
    xr[_slot(NSEG), :] = zh
    with jax.named_scope("sc_wait0"):
        c_x0.wait()
        c_m0.wait()
    if not cfg.get('dev'):
        for p in range(1, WIN):
            start_group(p)
    m0 = mem0[...].astype(F32)
    m00 = jnp.concatenate([m0, m0], axis=0)
    NPR = NPRE * HSEG

    def ldx(sl):
        return ub(x0[_half(sl), :]).astype(F32)

    def put(ref, r0, val):
        ref[r0 // 2:(r0 + val.shape[0]) // 2, :] = bu(val.astype(BF16))

    with jax.named_scope("sc_lnp"):
        for i in range(NPRE):
            put(lhsp, i * HSEG, _ln(ldx(_rows(LAG + i, n=HSEG))))
        put(lhsp, NPR + SEG, m00)
        put(lhs, 2 * SEG, m00)

    def step(t, a1, a2, h_on, r_on, first=False, usep=False, dummy=False, waitw=False, last=False, prepared=False, prep=False):
        r40 = lax.broadcasted_iota(jnp.int32, (40, 128), 0)
        c128 = lax.broadcasted_iota(jnp.int32, (40, 128), 1)
        hi = c128 >= 40
        j = jnp.where(hi, c128 - 40, c128)
        in0 = c128 < 40
        in1 = hi & (c128 < 80)
        lo_l = c128 < 64
        layers = [l for l, on in enumerate((a1, a2)) if on]
        nl = len(layers)
        nx = nl * SEG

        xs = {}
        f32l = nl == 1 and not first
        if a1:
            xs[0] = ldx(_rows(t))
            if prepared:
                pass
            elif first:
                put(lhsp, NPR, _ln(xs[0]))
            elif f32l:
                lhsf[0:SEG, :] = _ln(xs[0])
            elif usep:
                put(lhs, HSEG, _ln(xs[0][HSEG:]))
            else:
                put(lhs, 0, _ln(xs[0]))
        if a2:
            xs[1] = xr[_slot(t - LAG), :]
            if prepared:
                pass
            elif f32l:
                lhsf[0:SEG, :] = _ln(xs[1])
            else:
                put(lhs, SEG, _ln(xs[1]))
        if f32l:
            mrows = ub(lhs[SEG:, :]).astype(F32)
            lhsf[SEG:, :] = mrows[M * layers[0]:M * layers[0] + M]

        def L():
            if first:
                return ub(lhsp[...])
            if nl == 2:
                return ub(lhs[HSEG // 2:, :] if usep else lhs[...])
            return lhsf[...]

        def bd(a):
            z = jnp.zeros((40, 128), F32)
            a0, a1_, a2_ = a[:, 0:128], a[:, 128:256], a[:, 256:384]
            top = jnp.concatenate([a0, jnp.where(lo_l, a1_, z), z], axis=1)
            bot = jnp.concatenate([z, jnp.where(lo_l, z, a1_), a2_], axis=1)
            return jnp.concatenate([top, bot], axis=0).astype(BF16)

        def lrows(a, i):
            if nl == 1:
                return a[0:SEG + M]
            l = layers[i]
            return jnp.concatenate([a[SEG * i:SEG * i + SEG], a[nx + M * l:nx + M * l + M]], axis=0)

        def proj(m, p):
            if first:
                w = ub((wq, wk, wv)[m][prow(p), :])
                r = lax.dot_general(L(), w, NT_DIMS, preferred_element_type=F32)
                wn[m, p] = bu(w.T)
                if NPRE:
                    pre[m, p] = bu(r[0:NPR].astype(BF16))
                return r[NPR:]
            w = ub(wn[m, p])
            r = lax.dot_general(L(), w, NN_DIMS, preferred_element_type=F32)
            if usep:
                ps = t - LAG
                h2 = HSEG // 2
                pr_ = pl.ds(ps * h2, h2) if isinstance(ps, int) else pl.ds(pl.multiple_of(ps * h2, h2), h2)
                r = jnp.concatenate([ub(pre[m, p, pr_, :]).astype(F32), r], axis=0)
            return r

        def qk(q, k):
            return [lax.dot_general(lrows(q, i), bd(lrows(k, i)), NT_DIMS, preferred_element_type=F32)
                    for i in range(nl)]

        def softmax(sc):
            sc = jnp.concatenate([sc * SCALE, jnp.zeros((40, 48), F32)], axis=1)
            allowed = ((j >= 32) | (r40 >= 32) | (j <= r40)) & (c128 < 80)
            sc = jnp.where(allowed, sc, -1e9)
            m0_ = jnp.max(jnp.where(in0, sc, -jnp.inf), axis=-1, keepdims=True)
            m1_ = jnp.max(jnp.where(in1, sc, -jnp.inf), axis=-1, keepdims=True)
            e = jnp.exp(sc - jnp.where(hi, m1_, m0_))
            d0 = jnp.sum(jnp.where(in0, e, 0.0), axis=-1, keepdims=True)
            d1 = jnp.sum(jnp.where(in1, e, 0.0), axis=-1, keepdims=True)
            return (e * jnp.where(hi, 1.0 / d1, 1.0 / d0))[:, 0:80]

        def pv(prs, v):
            outs = [lax.dot_general(prs[i], bd(lrows(v, i)), NN_DIMS, preferred_element_type=F32)
                    for i in range(nl)]
            if nl == 1:
                return outs[0]
            return jnp.concatenate([outs[0][0:32], outs[1][0:32], outs[0][32:40], outs[1][32:40]], axis=0).astype(BF16)

        def oproj(o, p):
            w = ub(wo[prow(p), :])
            return lax.dot_general(o, w, NN_DIMS, preferred_element_type=F32)

        hsegs = [(l, t - 1 - LAG * l) for l in range(2) if h_on[l]]
        rsegs = [(l, t - 2 - LAG * l) for l in range(2) if r_on[l]]
        if last:
            rsegs = [(1, NSEG - 2), (1, NSEG - 1)]
        st = {}

        def B_h():
            if not hsegs:
                return
            xin = jnp.concatenate([xr[_slot(s), :] for _, s in hsegs], axis=0)
            zz = _ln(_ln(xin)).astype(BF16)
            st['h'] = jnp.dot(zz, ub(w1[...]), preferred_element_type=F32)

        def B_h2():
            if not hsegs:
                return
            h = _gelu(st['h'])
            for i, (l, s) in enumerate(hsegs):
                hv = h[i * SEG:(i + 1) * SEG]
                if dummy:
                    hv = jnp.where(_valid(s), hv, 0.0)
                hb[l, _slot(s), :] = hv

        def B_w2():
            if not rsegs:
                return
            if waitw:
                @pl.when(t == 1)
                def _():
                    c_w[1].wait()
                    c_w[2].wait()
                    c_w[3].wait()
            lane = lax.broadcasted_iota(jnp.int32, (SEG, D), 1)
            parts = []
            for l, s in rsegs:
                sc_ = jnp.clip(s, 0, NSEG - 1) if dummy else s
                win = hb[l, _slot(sc_, n=SEG + 16, off=-8), :]
                g0 = win[7:7 + SEG]
                g1 = win[9:9 + SEG]
                g2 = win[6:6 + SEG]
                g3 = win[10:10 + SEG]
                parts.append(jnp.where(lane < 320, jnp.where(lane < 160, g0, g1), jnp.where(lane < 480, g2, g3)))
            hc = jnp.concatenate(parts, axis=0).astype(BF16)
            st['hs'] = jnp.dot(hc, ub(w2[...]), preferred_element_type=F32)

        def B_w3():
            if not rsegs:
                return
            xres = jnp.concatenate([xr[_slot(s), :] for _, s in rsegs], axis=0)
            y1 = _ln(xres) + st['hs']
            st['y1x'] = xres + y1
            z1 = _ln(y1).astype(BF16)
            st['h3'] = jnp.dot(z1, ub(w3[...]), preferred_element_type=F32)

        def B_w4():
            if not rsegs:
                return
            h3 = _gelu(st['h3']).astype(BF16)
            ks = cfg.get('w4k', FF)
            if nl == 0:
                ks = FF
            st['h4'] = jnp.dot(h3[:, :ks], ub(w4[0:ks // 2, :]), preferred_element_type=F32)
            st['h3b'] = h3[:, ks:] if ks < FF else None

        def B_w4b():
            if not rsegs or st.get('h3b') is None:
                return
            ks = cfg['w4k']
            st['h4'] = st['h4'] + jnp.dot(st['h3b'], ub(w4[ks // 2:, :]), preferred_element_type=F32)

        def B_out():
            if not rsegs:
                return
            xnew = st['y1x'] + st['h4']
            st['xnew'] = xnew
            for i, (l, s) in enumerate(rsegs):
                if l == 0:
                    xr[_slot(s), :] = xnew[i * SEG:(i + 1) * SEG]
                else:
                    ob[_half(_slot(s)), :] = bu(xnew[i * SEG:(i + 1) * SEG].astype(BF16))
                    st.setdefault('out', []).append(s)

        chain = ((bh, B_h), (bh2, B_h2), (bw2, B_w2), (bw3, B_w3), (bw4, B_w4))

        def fill_at(key):
            for kk, f in chain:
                if kk == key:
                    f()

        def send_out():
            if 'out' not in st:
                return
            for s_ in st['out']:
                def go(s_=s_):
                    pltpu.make_async_copy(ob.at[_half(_slot(s_))], out_u.at[_half(_rows(s_))], osem).start()

                if dummy:
                    pl.when(s_ >= 0)(go)
                else:
                    go()

        if nl == 0:
            for _, f in chain:
                f()
            B_out()
            send_out()
            return

        if first:
            def pair_body(p, carry):
                sc_prev, v_prev, acc = carry
                for c in group(p):
                    c.wait()

                @pl.when(p + WIN < NP)
                def _():
                    for c in group(p + WIN):
                        c.start()

                @pl.when(p == cfg.get('bstart', NP - 1))
                def _():
                    start_group(NP)

                q = proj(0, p)
                k = proj(1, p)
                o = pv([softmax(sc_prev)], v_prev)
                v = proj(2, p)
                sc = qk(q, k)
                acc = acc + oproj(o, jnp.maximum(p - 1, 0))
                return sc[0], v[0:SEG + M], acc

            init = (jnp.zeros((SEG + M, 80), F32), jnp.zeros((SEG + M, PW), F32), jnp.zeros((SEG + M, D), F32))
            sc_l, v_l, acc = lax.fori_loop(0, NP, pair_body, init)
            acc = acc + oproj(pv([softmax(sc_l)], v_l), NP - 1)
        else:
            acc = None
            q = proj(0, 0); k = proj(1, 0); v = proj(2, 0)
            sc = qk(q, k)
            for p in range(NP):
                fill_at(p)
                if p + 1 < NP:
                    qn = proj(0, p + 1)
                    kn = proj(1, p + 1)
                prs = [softmax(sc[i]) for i in range(nl)]
                o = pv(prs, v)
                if p + 1 < NP:
                    v = proj(2, p + 1)
                    sc = qk(qn, kn)
                else:
                    fill_at(100)
                r = oproj(o, p)
                acc = r if acc is None else acc + r
            fill_at(101)
            B_w4b()
            B_out()

        if a1:
            xr[_slot(t), :] = xs[0] + acc[0:SEG]
        if a2:
            i = layers.index(1)
            xr[_slot(t - LAG), :] = xs[1] + acc[i * SEG:(i + 1) * SEG]
        if nl == 2:
            mm = acc[nx:]
        elif layers[0] == 0:
            mm = jnp.concatenate([acc[nx:], m0], axis=0)
        else:
            mm = jnp.concatenate([m0, acc[nx:]], axis=0)
        if prep:
            tn = min(t + 1, NSEG - 1) if isinstance(t, int) else jnp.minimum(t + 1, NSEG - 1)
            if prep == 'single1':
                lhsf[0:SEG, :] = _ln(ldx(_rows(tn)))
            elif prep == 'single2':
                lhsf[0:SEG, :] = _ln(st['xnew'][0:SEG])
            else:
                put(lhs, 0, _ln(ldx(_rows(tn))))
                put(lhs, SEG, _ln(st['xnew'][0:SEG]))
        put(lhs, 2 * SEG, mm)
        send_out()

    def flags(t):
        a1 = 0 <= t < NSEG
        a2 = 0 <= t - LAG < NSEG
        h_on = tuple(0 <= t - 1 - LAG * l < NSEG for l in range(2))
        r_on = tuple(0 <= t - 2 - LAG * l < NSEG for l in range(2))
        return a1, a2, h_on, r_on

    def scope(name):
        return jax.named_scope(name)

    PREP = cfg.get('prep', True)
    PREPS = cfg.get('preps', True)
    if cfg.get('bench'):
        for p in range(1 if not cfg.get('dev') else NP + 1, NP + 1):
            if p >= WIN:
                start_group(p)
        for p in range(NP):
            for c in group(p):
                c.wait()
        for c in c_w:
            c.wait()
        c_x1.wait()
        wn[...] = jnp.zeros(wn.shape, U32)
        xr[...] = jnp.zeros(xr.shape, F32)
        hb[...] = jnp.zeros(hb.shape, F32)
        lax.fori_loop(18, NSEG, lambda t, c: (step(t, True, True, (True, True), (True, True), prepared=PREP, prep=PREP), c)[1], 0)
        cp = pltpu.make_async_copy(ob.at[pl.ds(SEG // 2, 23 * SEG)], out_u.at[pl.ds(0, 23 * SEG)], osem)
        cp.wait()
        return
    with scope("sc_t0"):
        step(0, *flags(0), first=True, prep=('single1' if PREPS else False))
    ON, OFF = True, False

    def loop(name, lo, hi, *fl, **kw):
        with scope(name):
            lax.fori_loop(lo, hi, lambda t, c: (step(t, *fl, **kw), c)[1], 0)

    mode = cfg.get('mode', 'loops')
    if mode == 'loops':
        if cfg.get('head', 'loop') == 'loop':
            for c in c_w:
                c.wait()
            loop("sc_head", 1, LAG, ON, OFF, (ON, OFF), (ON, OFF), dummy=True)
        elif cfg['head'] == 'loopw':
            c_w[0].wait()
            loop("sc_head", 1, LAG, ON, OFF, (ON, OFF), (ON, OFF), dummy=True, waitw=True)
        else:
            for t in range(1, LAG):
                if t == 1:
                    c_w[0].wait()
                if t == 2:
                    c_w[1].wait()
                    c_w[2].wait()
                    c_w[3].wait()
                with scope(f"sc_t{t}"):
                    step(t, *flags(t), prepared=PREPS,
                         prep=(PREP if t == LAG - 1 else ('single1' if PREPS else False)))
        T1 = max(LAG, LAG + NPRE)
        loop("sc_loopP", LAG, T1, ON, ON, (ON, ON), (ON, ON), usep=True, dummy=True, prepared=PREP, prep=PREP)
        c_x1.wait()
        loop("sc_loop", T1, NSEG, ON, ON, (ON, ON), (ON, ON), prepared=PREP, prep=PREP)
        if cfg.get('tail', 'loop') == 'loop':
            loop("sc_tail", NSEG, NSEG + LAG, OFF, ON, (ON, ON), (ON, ON), dummy=True)
        else:
            for t in range(NSEG, NSEG + LAG):
                with scope(f"sc_t{t}"):
                    step(t, *flags(t), prepared=(PREPS and t > NSEG),
                         prep=('single2' if PREPS and t < NSEG + LAG - 1 else False))
    if cfg.get('mergelast', True):
        with scope("sc_last"):
            step(NSEG + LAG, *flags(NSEG + LAG), last=True)
    else:
        for t in range(NSEG + LAG, NSEG + LAG + 2):
            with scope(f"sc_t{t}"):
                step(t, *flags(t))
    pltpu.make_async_copy(ob.at[pl.ds(SEG // 2, S // 2)], out_u, osem).wait()


def make(bpos=(1, 2, 3, 15, 100), out_overlap=True, npre=16, win=2, **kw):
    cfg = dict(bpos=tuple(bpos), out_overlap=out_overlap, npre=npre, win=win, **kw)

    def fn(A_x, A_mem0, A_Wq, A_Wk, A_Wv, A_Wo, A_seg_len, B_x, B_w1, B_w2, B_w3, B_w4):
        x = A_x.reshape(S, D)
        mem0 = A_mem0.reshape(M, D)
        tr = lambda w: jnp.transpose(w, (1, 2, 0)).reshape(HD, D)
        wq, wk, wv = tr(A_Wq), tr(A_Wk), tr(A_Wv)
        wo = A_Wo.reshape(HD, D)
        hbm = pl.BlockSpec(memory_space=pltpu.HBM)
        out = pl.pallas_call(
            functools.partial(kernel, cfg=cfg),
            out_shape=jax.ShapeDtypeStruct((S, D), BF16),
            in_specs=[hbm] * 10,
            out_specs=hbm,
            scratch_shapes=[
                pltpu.VMEM((S // 2, D), U32), pltpu.VMEM((M, D), BF16),
                pltpu.VMEM((HD // 2, D), U32), pltpu.VMEM((HD // 2, D), U32), pltpu.VMEM((HD // 2, D), U32),
                pltpu.VMEM((HD // 2, D), U32),
                pltpu.VMEM((D // 2, D), U32), pltpu.VMEM((D // 2, D), U32),
                pltpu.VMEM((D // 2, FF), U32), pltpu.VMEM((FF // 2, D), U32),
                pltpu.VMEM((S + 2 * SEG, D), F32),
                pltpu.VMEM((2, S + 2 * SEG, D), F32),
                pltpu.VMEM((S // 2 + SEG, D), U32),
                pltpu.VMEM((SEG + M, D), U32),
                pltpu.VMEM(((cfg['npre'] * HSEG + SEG + 2 * M) // 2, D), U32),
                pltpu.VMEM((3, NP, max(cfg['npre'], 1) * HSEG // 2, PW), U32),
                pltpu.VMEM((3, NP, D // 2, PW), U32),
                pltpu.VMEM((SEG + M, D), F32),
                pltpu.SemaphoreType.DMA((7,)),
                pltpu.SemaphoreType.DMA((NP,)),
                pltpu.SemaphoreType.DMA,
            ],
            compiler_params=pltpu.CompilerParams(vmem_limit_bytes=110 * 1024 * 1024),
        )(x, mem0, wq, wk, wv, wo, B_w1, B_w2, B_w3, B_w4)
        return out.reshape(1, S, D)
    return fn


_fn = make(npre=16, head="unroll", tail="unroll")


@functools.partial(jax.jit, static_argnames=["A_seg_len"])
def pallas_interleave_layers__memory_aug_recurrent_mem_tr__mixer_s_mlp__prompt_kernel(
        A_x, A_mem0, A_Wq, A_Wk, A_Wv, A_Wo, A_seg_len, B_x, B_w1, B_w2, B_w3, B_w4):
    assert A_seg_len == SEG
    return _fn(A_x, A_mem0, A_Wq, A_Wk, A_Wv, A_Wo, A_seg_len, B_x, B_w1, B_w2, B_w3, B_w4)
```

```python
import functools

import jax
import jax.numpy as jnp
from jax import lax
from jax.experimental import pallas as pl
from jax.experimental.pallas import tpu as pltpu

F32 = jnp.float32
BF16 = jnp.bfloat16
U32 = jnp.uint32

S, D, H, DH, M, SEG, FF = 2048, 640, 32, 192, 8, 32, 1536
NSEG = S // SEG
HD = H * DH
NP = H // 2
PW = 2 * DH
LAG = 3
HALO = 8
NPRE = 16
PRE_ROWS = 16
WIN = 2
SCALE = float(DH) ** -0.5
NT_DIMS = (((1,), (1,)), ((), ()))
NN_DIMS = (((1,), (0,)), ((), ()))


def _ln(x):
    m = jnp.mean(x, axis=-1, keepdims=True)
    c = x - m
    v = jnp.mean(c * c, axis=-1, keepdims=True)
    return c * lax.rsqrt(v + 1e-5)


def _gelu(x):
    return 0.5 * x * (1.0 + jnp.tanh(0.7978845608028654 * (x + 0.044715 * (x * x * x))))


def _dot(a, b, dims=NN_DIMS):
    return lax.dot_general(a, b, dims, preferred_element_type=F32)


def _ub(x):
    return pltpu.bitcast(x, BF16)


def _bu(x):
    return pltpu.bitcast(x.astype(BF16), U32)


def _ds(i, unit, n, off=0):
    if isinstance(i, int):
        return pl.ds(i * unit + off, n)
    return pl.ds(pl.multiple_of(i * unit, unit) + off, n)


def _kernel(x_hbm, mem0_hbm, wq_hbm, wk_hbm, wv_hbm, wo_hbm, w1_hbm, w2_hbm, w3_hbm, w4_hbm,
            out_hbm,
            x0, mem0, wq, wk, wv, wo, w1, w2, w3, w4,
            xr, hb, ob, lhs, lhs0, lhsf, pre, wn, sems, psems, osem):
    HS, PW2 = SEG // 2, PW // 2
    NPR = NPRE * PRE_ROWS

    xu, out_u = x_hbm.bitcast(U32), out_hbm.bitcast(U32)
    xfirst = (LAG + NPRE + 1) * HS
    c_x0 = pltpu.make_async_copy(xu.at[pl.ds(0, xfirst)], x0.at[pl.ds(0, xfirst)], sems.at[0])
    c_m0 = pltpu.make_async_copy(mem0_hbm, mem0, sems.at[1])
    c_x1 = pltpu.make_async_copy(xu.at[pl.ds(xfirst, S // 2 - xfirst)],
                                 x0.at[pl.ds(xfirst, S // 2 - xfirst)], sems.at[2])
    c_w = [pltpu.make_async_copy(s.bitcast(U32), d, sems.at[3 + i]) for i, (s, d) in
           enumerate(((w1_hbm, w1), (w2_hbm, w2), (w3_hbm, w3), (w4_hbm, w4)))]

    def group(p):
        rows = _ds(p, PW2, PW2)
        return [pltpu.make_async_copy(s.bitcast(U32).at[rows], d.at[rows], psems.at[p])
                for s, d in ((wq_hbm, wq), (wk_hbm, wk), (wv_hbm, wv), (wo_hbm, wo))]

    c_x0.start()
    c_m0.start()
    for c in group(0):
        c.start()

    zh = jnp.zeros((HALO, D), F32)
    for l in range(2):
        hb[l, 0:HALO, :] = zh
        hb[l, HALO + S:, :] = zh

    c_x0.wait()
    c_m0.wait()
    for p in range(1, WIN):
        for c in group(p):
            c.start()

    def x_rows(s, n=SEG):
        return _ub(x0[_ds(s, HS, n // 2), :]).astype(F32)

    def put(ref, r0, val):
        ref[r0 // 2:(r0 + val.shape[0]) // 2, :] = _bu(val)

    m0 = mem0[...].astype(F32)
    m00 = jnp.concatenate([m0, m0], axis=0)
    for i in range(NPRE):
        put(lhs0, i * PRE_ROWS, _ln(x_rows(LAG + i, PRE_ROWS)))
    put(lhs0, NPR + SEG, m00)
    put(lhs, 2 * SEG, m00)

    def step(t, a_on, hsegs, rsegs, nxt=None, first=False, use_pre=False, mem_out=True):
        layers = [l for l in range(2) if a_on[l]]
        nl = len(layers)
        nx = nl * SEG
        nq = SEG + M if mem_out else SEG
        NK = SEG + M
        row = lax.broadcasted_iota(jnp.int32, (nq, 128), 0)
        col = lax.broadcasted_iota(jnp.int32, (nq, 128), 1)
        hi = col >= NK
        key = jnp.where(hi, col - NK, col)
        in0 = col < NK
        in1 = hi & (col < 2 * NK)
        allowed = ((key >= SEG) | (row >= SEG) | (key <= row)) & (col < 2 * NK)
        lo_half = lax.broadcasted_iota(jnp.int32, (NK, 128), 1) < 64

        xs = []
        if a_on[0]:
            xs.append(x_rows(t))
        if a_on[1]:
            xs.append(xr[_ds(t - LAG, SEG, SEG), :])
        if first:
            put(lhs0, NPR, _ln(xs[0]))
        elif nl == 1:
            l = layers[0]
            lhsf[SEG:, :] = _ub(lhs[SEG:, :]).astype(F32)[M * l:M * l + M]

        def lhs_rows():
            if first:
                return _ub(lhs0[...])
            if nl == 2:
                return _ub(lhs[PRE_ROWS // 2:, :] if use_pre else lhs[...])
            return lhsf[...]

        def proj(m, p):
            if first:
                w = _ub((wq, wk, wv)[m][_ds(p, PW2, PW2), :])
                r = _dot(lhs_rows(), w, NT_DIMS)
                wn[m, p] = pltpu.bitcast(w.T, U32)
                pre[m, p] = _bu(r[0:NPR])
                return r[NPR:]
            rows = lhs_rows() if (mem_out or m > 0) else lhsf[0:SEG, :]
            r = _dot(rows, _ub(wn[m, p]))
            if use_pre:
                r = jnp.concatenate(
                    [_ub(pre[m, p, _ds(t - LAG, PRE_ROWS // 2, PRE_ROWS // 2), :]).astype(F32), r], axis=0)
            return r

        def sel(a, i, n=NK):
            if nl == 1:
                return a[0:n]
            l = layers[i]
            return jnp.concatenate([a[SEG * i:SEG * i + SEG], a[nx + M * l:nx + M * l + M]], axis=0)

        def blockdiag(a):
            z = jnp.zeros((NK, 128), F32)
            a0, a1, a2 = a[:, 0:128], a[:, 128:256], a[:, 256:384]
            top = jnp.concatenate([a0, jnp.where(lo_half, a1, z), z], axis=1)
            bot = jnp.concatenate([z, jnp.where(lo_half, z, a1), a2], axis=1)
            return jnp.concatenate([top, bot], axis=0).astype(BF16)

        def scores(q, k):
            return [_dot(sel(q, i, nq), blockdiag(sel(k, i)), NT_DIMS) for i in range(nl)]

        def softmax(sc):
            sc = jnp.concatenate([sc * SCALE, jnp.zeros((nq, 128 - 2 * NK), F32)], axis=1)
            sc = jnp.where(allowed, sc, -1e9)
            mx0 = jnp.max(jnp.where(in0, sc, -jnp.inf), axis=-1, keepdims=True)
            mx1 = jnp.max(jnp.where(in1, sc, -jnp.inf), axis=-1, keepdims=True)
            e = jnp.exp(sc - jnp.where(hi, mx1, mx0))
            d0 = jnp.sum(jnp.where(in0, e, 0.0), axis=-1, keepdims=True)
            d1 = jnp.sum(jnp.where(in1, e, 0.0), axis=-1, keepdims=True)
            return (e * jnp.where(hi, 1.0 / d1, 1.0 / d0))[:, 0:2 * NK]

        def values(prs, v):
            o = [_dot(prs[i], blockdiag(sel(v, i))) for i in range(nl)]
            if nl == 1:
                return o[0]
            return jnp.concatenate([o[0][0:SEG], o[1][0:SEG], o[0][SEG:], o[1][SEG:]], axis=0).astype(BF16)

        def oproj(o, p):
            return _dot(o, _ub(wo[_ds(p, PW2, PW2), :]))

        st = {}

        def mlp_h():
            xin = jnp.concatenate([xr[_ds(s, SEG, SEG), :] for _, s in hsegs], axis=0)
            st['h'] = _dot(_ln(_ln(xin)).astype(BF16), _ub(w1[...]))

        def mlp_h_store():
            h = _gelu(st['h'])
            for i, (l, s) in enumerate(hsegs):
                hb[l, _ds(s, SEG, SEG, HALO), :] = h[i * SEG:(i + 1) * SEG]

        def mlp_w2():
            lane = lax.broadcasted_iota(jnp.int32, (SEG, D), 1)
            c = D // 4
            parts = []
            for l, s in rsegs:
                win = hb[l, _ds(s, SEG, SEG + 2 * HALO), :]
                g0 = win[HALO - 1:HALO - 1 + SEG]
                g1 = win[HALO + 1:HALO + 1 + SEG]
                g2 = win[HALO - 2:HALO - 2 + SEG]
                g3 = win[HALO + 2:HALO + 2 + SEG]
                parts.append(jnp.where(lane < 2 * c, jnp.where(lane < c, g0, g1),
                                       jnp.where(lane < 3 * c, g2, g3)))
            st['hs'] = _dot(jnp.concatenate(parts, axis=0).astype(BF16), _ub(w2[...]))

        def mlp_w3():
            xres = jnp.concatenate([xr[_ds(s, SEG, SEG), :] for _, s in rsegs], axis=0)
            y1 = _ln(xres) + st['hs']
            st['y1x'] = xres + y1
            st['h3'] = _dot(_ln(y1).astype(BF16), _ub(w3[...]))

        def mlp_w4():
            st['h4'] = _dot(_gelu(st['h3']).astype(BF16), _ub(w4[...]))

        def mlp_out():
            xnew = st['y1x'] + st['h4']
            st['xnew'] = xnew
            for i, (l, s) in enumerate(rsegs):
                if l == 0:
                    xr[_ds(s, SEG, SEG), :] = xnew[i * SEG:(i + 1) * SEG]
                else:
                    ob[_ds(s, HS, HS), :] = _bu(xnew[i * SEG:(i + 1) * SEG])

        def mlp_send():
            for l, s in rsegs:
                if l == 1:
                    pltpu.make_async_copy(ob.at[_ds(s, HS, HS)], out_u.at[_ds(s, HS, HS)], osem).start()

        slots = {1: (hsegs, mlp_h), 2: (hsegs, mlp_h_store), 3: (rsegs, mlp_w2),
                 NP - 1: (rsegs, mlp_w3), NP: (rsegs, mlp_w4)}

        def mlp_at(key):
            segs, f = slots.get(key, (None, None))
            if segs:
                f()

        if nl == 0:
            for key in sorted(slots):
                mlp_at(key)
            mlp_out()
            mlp_send()
            return

        if first:
            def pair_body(p, carry):
                sc_prev, v_prev, acc = carry
                for c in group(p):
                    c.wait()

                @pl.when(p + WIN < NP)
                def _():
                    for c in group(p + WIN):
                        c.start()

                @pl.when(p == NP - 1)
                def _():
                    for c in c_w:
                        c.start()

                q = proj(0, p)
                k = proj(1, p)
                o = values([softmax(sc_prev)], v_prev)
                v = proj(2, p)
                sc = scores(q, k)
                acc = acc + oproj(o, jnp.maximum(p - 1, 0))
                return sc[0], v[0:NK], acc

            init = (jnp.zeros((NK, 2 * NK), F32), jnp.zeros((NK, PW), F32), jnp.zeros((NK, D), F32))
            sc_l, v_l, acc = lax.fori_loop(0, NP, pair_body, init)
            acc = acc + oproj(values([softmax(sc_l)], v_l), NP - 1)
        else:
            acc = None
            q = proj(0, 0)
            k = proj(1, 0)
            v = proj(2, 0)
            sc = scores(q, k)
            for p in range(NP):
                mlp_at(p)
                if p + 1 < NP:
                    qn = proj(0, p + 1)
                    kn = proj(1, p + 1)
                prs = [softmax(sc[i]) for i in range(nl)]
                o = values(prs, v)
                if p + 1 < NP:
                    v = proj(2, p + 1)
                    sc = scores(qn, kn)
                else:
                    mlp_at(NP)
                r = oproj(o, p)
                acc = r if acc is None else acc + r
            if rsegs:
                mlp_out()

        if a_on[0]:
            xr[_ds(t, SEG, SEG), :] = xs[0] + acc[0:SEG]
        if a_on[1]:
            i = layers.index(1)
            xr[_ds(t - LAG, SEG, SEG), :] = xs[i] + acc[i * SEG:(i + 1) * SEG]
        if nxt is not None:
            tn = min(t + 1, NSEG - 1) if isinstance(t, int) else jnp.minimum(t + 1, NSEG - 1)
            if nxt == 'layer0':
                lhsf[0:SEG, :] = _ln(x_rows(tn))
            elif nxt == 'layer1':
                lhsf[0:SEG, :] = _ln(st['xnew'][0:SEG])
            else:
                put(lhs, 0, _ln(x_rows(tn)))
                put(lhs, SEG, _ln(st['xnew'][0:SEG]))
        if mem_out:
            if nl == 2:
                mm = acc[nx:]
            elif layers[0] == 0:
                mm = jnp.concatenate([acc[nx:], m0], axis=0)
            else:
                mm = jnp.concatenate([m0, acc[nx:]], axis=0)
            put(lhs, 2 * SEG, mm)
        mlp_send()

    def mlp_segs(t):
        hs = [(l, t - 1 - LAG * l) for l in range(2)]
        rs = [(l, t - 2 - LAG * l) for l in range(2)]
        if isinstance(t, int):
            hs = [(l, s) for l, s in hs if 0 <= s < NSEG]
            rs = [(l, s) for l, s in rs if 0 <= s < NSEG]
        return hs, rs

    BOTH, L0, L1 = (True, True), (True, False), (False, True)

    step(0, L0, *mlp_segs(0), nxt='layer0', first=True)
    c_w[0].wait()
    step(1, L0, *mlp_segs(1), nxt='layer0')
    c_w[1].wait()
    c_w[2].wait()
    c_w[3].wait()
    step(2, L0, *mlp_segs(2), nxt='both')
    step(LAG, BOTH, *mlp_segs(LAG), nxt='both', use_pre=True)
    step(LAG + 1, BOTH, *mlp_segs(LAG + 1), nxt='both', use_pre=True)

    def loop(lo, hi, **kw):
        def body(t, c):
            step(t, BOTH, *mlp_segs(t), nxt='both', **kw)
            return c
        lax.fori_loop(lo, hi, body, 0)

    c_x1.start()
    loop(LAG + 2, LAG + NPRE, use_pre=True)
    c_x1.wait()
    loop(LAG + NPRE, NSEG)
    t = NSEG
    hs, rs = mlp_segs(t)
    lhsf[0:SEG, :] = _ln(xr[_ds(t - LAG, SEG, SEG), :])
    step(t, L1, hs, rs, nxt='layer1')
    step(t + 1, L1, *mlp_segs(t + 1), nxt='layer1')
    step(t + 2, L1, *mlp_segs(t + 2), mem_out=False)
    step(t + 3, (False, False), [(1, NSEG - 1)], [(1, NSEG - 2), (1, NSEG - 1)])
    pltpu.make_async_copy(ob, out_u, osem).wait()


def _call(A_x, A_mem0, A_Wq, A_Wk, A_Wv, A_Wo, B_w1, B_w2, B_w3, B_w4):
    x = A_x.reshape(S, D)
    mem0 = A_mem0.reshape(M, D)
    tr = lambda w: jnp.transpose(w, (1, 2, 0)).reshape(HD, D)
    hbm = pl.BlockSpec(memory_space=pltpu.HBM)
    out = pl.pallas_call(
        _kernel,
        out_shape=jax.ShapeDtypeStruct((S, D), BF16),
        in_specs=[hbm] * 10,
        out_specs=hbm,
        scratch_shapes=[
            pltpu.VMEM((S // 2, D), U32),
            pltpu.VMEM((M, D), BF16),
            pltpu.VMEM((HD // 2, D), U32),
            pltpu.VMEM((HD // 2, D), U32),
            pltpu.VMEM((HD // 2, D), U32),
            pltpu.VMEM((HD // 2, D), U32),
            pltpu.VMEM((D // 2, D), U32),
            pltpu.VMEM((D // 2, D), U32),
            pltpu.VMEM((D // 2, FF), U32),
            pltpu.VMEM((FF // 2, D), U32),
            pltpu.VMEM((S, D), F32),
            pltpu.VMEM((2, S + 2 * HALO, D), F32),
            pltpu.VMEM((S // 2, D), U32),
            pltpu.VMEM((SEG + M, D), U32),
            pltpu.VMEM(((NPRE * PRE_ROWS + SEG + 2 * M) // 2, D), U32),
            pltpu.VMEM((SEG + M, D), F32),
            pltpu.VMEM((3, NP, NPRE * PRE_ROWS // 2, PW), U32),
            pltpu.VMEM((3, NP, D // 2, PW), U32),
            pltpu.SemaphoreType.DMA((7,)),
            pltpu.SemaphoreType.DMA((NP,)),
            pltpu.SemaphoreType.DMA,
        ],
        compiler_params=pltpu.CompilerParams(vmem_limit_bytes=110 * 1024 * 1024),
    )(x, mem0, tr(A_Wq), tr(A_Wk), tr(A_Wv), A_Wo.reshape(HD, D), B_w1, B_w2, B_w3, B_w4)
    return out.reshape(1, S, D)


@functools.partial(jax.jit, static_argnames=["A_seg_len"])
def pallas_interleave_layers__memory_aug_recurrent_mem_tr__mixer_s_mlp__prompt_kernel(
        A_x, A_mem0, A_Wq, A_Wk, A_Wv, A_Wo, A_seg_len, B_x, B_w1, B_w2, B_w3, B_w4):
    assert A_seg_len == SEG and A_x.shape == (1, S, D) and A_Wq.shape == (D, H, DH)
    assert A_mem0.shape == (1, M, D) and B_w3.shape == (D, FF)
    del B_x
    return _call(A_x, A_mem0, A_Wq, A_Wk, A_Wv, A_Wo, B_w1, B_w2, B_w3, B_w4)
```

```python
import functools

import jax
import jax.numpy as jnp
from jax import lax
from jax.experimental import pallas as pl
from jax.experimental.pallas import tpu as pltpu

F32 = jnp.float32
BF16 = jnp.bfloat16
U32 = jnp.uint32

S, D, H, DH, M, SEG, FF = 2048, 640, 32, 192, 8, 32, 1536
NSEG = S // SEG
HD = H * DH
NP = H // 2
PW = 2 * DH
LAG = 3
HALO = 8
NPRE = 17
PRE_ROWS = 16
WIN = 2
SCALE = float(DH) ** -0.5
NT_DIMS = (((1,), (1,)), ((), ()))
NN_DIMS = (((1,), (0,)), ((), ()))


def _ln(x):
    m = jnp.mean(x, axis=-1, keepdims=True)
    c = x - m
    v = jnp.mean(c * c, axis=-1, keepdims=True)
    return c * lax.rsqrt(v + 1e-5)


def _gelu(x):
    return 0.5 * x * (1.0 + jnp.tanh(0.7978845608028654 * (x + 0.044715 * (x * x * x))))


def _dot(a, b, dims=NN_DIMS):
    return lax.dot_general(a, b, dims, preferred_element_type=F32)


def _ub(x):
    return pltpu.bitcast(x, BF16)


def _bu(x):
    return pltpu.bitcast(x.astype(BF16), U32)


def _ds(i, unit, n, off=0):
    if isinstance(i, int):
        return pl.ds(i * unit + off, n)
    return pl.ds(pl.multiple_of(i * unit, unit) + off, n)


def _kernel(x_hbm, mem0_hbm, wq_hbm, wk_hbm, wv_hbm, wo_hbm, w1_hbm, w2_hbm, w3_hbm, w4_hbm,
            out_hbm,
            x0, mem0, wq, wk, wv, wo, w1, w2, w3, w4,
            xr, hb, ob, lhs, lhs0, lhsf, pre, wn, csc, cv, cacc, sems, psems, osem):
    HS, PW2 = SEG // 2, PW // 2
    NPR = NPRE * PRE_ROWS

    xu, out_u = x_hbm.bitcast(U32), out_hbm.bitcast(U32)
    xfirst = (LAG + NPRE + 1) * HS
    c_x0 = pltpu.make_async_copy(xu.at[pl.ds(0, xfirst)], x0.at[pl.ds(0, xfirst)], sems.at[0])
    c_m0 = pltpu.make_async_copy(mem0_hbm, mem0, sems.at[1])
    c_x1 = pltpu.make_async_copy(xu.at[pl.ds(xfirst, S // 2 - xfirst)],
                                 x0.at[pl.ds(xfirst, S // 2 - xfirst)], sems.at[2])
    c_w = [pltpu.make_async_copy(s.bitcast(U32), d, sems.at[3 + i]) for i, (s, d) in
           enumerate(((w1_hbm, w1), (w2_hbm, w2), (w3_hbm, w3), (w4_hbm, w4)))]

    def group(p):
        rows = _ds(p, PW2, PW2)
        return [pltpu.make_async_copy(s.bitcast(U32).at[rows], d.at[rows], psems.at[p])
                for s, d in ((wq_hbm, wq), (wk_hbm, wk), (wv_hbm, wv), (wo_hbm, wo))]

    c_x0.start()
    c_m0.start()
    for c in group(0):
        c.start()

    zh = jnp.zeros((HALO, D), F32)
    for l in range(2):
        hb[l, 0:HALO, :] = zh
        hb[l, HALO + S:, :] = zh

    c_x0.wait()
    c_m0.wait()
    for p in range(1, WIN):
        for c in group(p):
            c.start()

    def x_rows(s, n=SEG):
        return _ub(x0[_ds(s, HS, n // 2), :]).astype(F32)

    def put(ref, r0, val):
        ref[r0 // 2:(r0 + val.shape[0]) // 2, :] = _bu(val)

    m0 = mem0[...].astype(F32)
    m00 = jnp.concatenate([m0, m0], axis=0)
    for i in range(NPRE):
        put(lhs0, i * PRE_ROWS, _ln(x_rows(LAG + i, PRE_ROWS)))
    put(lhs0, NPR + SEG, m00)
    put(lhs, 2 * SEG, m00)

    def step(t, a_on, hsegs, rsegs, nxt=None, first=False, use_pre=False, mem_out=True):
        layers = [l for l in range(2) if a_on[l]]
        nl = len(layers)
        nx = nl * SEG
        nq = SEG + M if mem_out else SEG
        NK = SEG + M
        row = lax.broadcasted_iota(jnp.int32, (nq, 128), 0)
        col = lax.broadcasted_iota(jnp.int32, (nq, 128), 1)
        hi = col >= NK
        key = jnp.where(hi, col - NK, col)
        in0 = col < NK
        in1 = hi & (col < 2 * NK)
        allowed = ((key >= SEG) | (row >= SEG) | (key <= row)) & (col < 2 * NK)
        lo_half = lax.broadcasted_iota(jnp.int32, (NK, 128), 1) < 64

        xs = []
        if a_on[0]:
            xs.append(x_rows(t))
        if a_on[1]:
            xs.append(xr[_ds(t - LAG, SEG, SEG), :])
        if first:
            put(lhs0, NPR, _ln(xs[0]))
        elif nl == 1:
            l = layers[0]
            lhsf[SEG:, :] = _ub(lhs[SEG:, :]).astype(F32)[M * l:M * l + M]

        def lhs_rows():
            if first:
                return _ub(lhs0[...])
            if nl == 2:
                return _ub(lhs[PRE_ROWS // 2:, :] if use_pre else lhs[...])
            return lhsf[...]

        def proj(m, p):
            if first:
                w = _ub((wq, wk, wv)[m][_ds(p, PW2, PW2), :])
                r = _dot(lhs_rows(), w, NT_DIMS)
                wn[m, p] = pltpu.bitcast(w.T, U32)
                pre[m, p] = _bu(r[0:NPR])
                return r[NPR:]
            rows = lhs_rows() if (mem_out or m > 0) else lhsf[0:SEG, :]
            r = _dot(rows, _ub(wn[m, p]))
            if use_pre:
                r = jnp.concatenate(
                    [_ub(pre[m, p, _ds(t - LAG, PRE_ROWS // 2, PRE_ROWS // 2), :]).astype(F32), r], axis=0)
            return r

        def sel(a, i, n=NK):
            if nl == 1:
                return a[0:n]
            l = layers[i]
            return jnp.concatenate([a[SEG * i:SEG * i + SEG], a[nx + M * l:nx + M * l + M]], axis=0)

        def blockdiag(a):
            z = jnp.zeros((NK, 128), F32)
            a0, a1, a2 = a[:, 0:128], a[:, 128:256], a[:, 256:384]
            top = jnp.concatenate([a0, jnp.where(lo_half, a1, z), z], axis=1)
            bot = jnp.concatenate([z, jnp.where(lo_half, z, a1), a2], axis=1)
            return jnp.concatenate([top, bot], axis=0).astype(BF16)

        def scores(q, k):
            return [_dot(sel(q, i, nq), blockdiag(sel(k, i)), NT_DIMS) for i in range(nl)]

        def softmax(sc):
            sc = jnp.concatenate([sc * SCALE, jnp.zeros((nq, 128 - 2 * NK), F32)], axis=1)
            sc = jnp.where(allowed, sc, -1e9)
            mx0 = jnp.max(jnp.where(in0, sc, -jnp.inf), axis=-1, keepdims=True)
            mx1 = jnp.max(jnp.where(in1, sc, -jnp.inf), axis=-1, keepdims=True)
            e = jnp.exp(sc - jnp.where(hi, mx1, mx0))
            d0 = jnp.sum(jnp.where(in0, e, 0.0), axis=-1, keepdims=True)
            d1 = jnp.sum(jnp.where(in1, e, 0.0), axis=-1, keepdims=True)
            return (e * jnp.where(hi, 1.0 / d1, 1.0 / d0))[:, 0:2 * NK]

        def values(prs, v):
            o = [_dot(prs[i], blockdiag(sel(v, i))) for i in range(nl)]
            if nl == 1:
                return o[0]
            return jnp.concatenate([o[0][0:SEG], o[1][0:SEG], o[0][SEG:], o[1][SEG:]], axis=0).astype(BF16)

        def oproj(o, p):
            return _dot(o, _ub(wo[_ds(p, PW2, PW2), :]))

        st = {}

        def mlp_h():
            xin = jnp.concatenate([xr[_ds(s, SEG, SEG), :] for _, s in hsegs], axis=0)
            st['h'] = _dot(_ln(_ln(xin)).astype(BF16), _ub(w1[...]))

        def mlp_h_store():
            h = _gelu(st['h'])
            for i, (l, s) in enumerate(hsegs):
                hb[l, _ds(s, SEG, SEG, HALO), :] = h[i * SEG:(i + 1) * SEG]

        def mlp_w2():
            lane = lax.broadcasted_iota(jnp.int32, (SEG, D), 1)
            c = D // 4
            parts = []
            for l, s in rsegs:
                win = hb[l, _ds(s, SEG, SEG + 2 * HALO), :]
                g0 = win[HALO - 1:HALO - 1 + SEG]
                g1 = win[HALO + 1:HALO + 1 + SEG]
                g2 = win[HALO - 2:HALO - 2 + SEG]
                g3 = win[HALO + 2:HALO + 2 + SEG]
                parts.append(jnp.where(lane < 2 * c, jnp.where(lane < c, g0, g1),
                                       jnp.where(lane < 3 * c, g2, g3)))
            st['hs'] = _dot(jnp.concatenate(parts, axis=0).astype(BF16), _ub(w2[...]))

        def mlp_w3():
            xres = jnp.concatenate([xr[_ds(s, SEG, SEG), :] for _, s in rsegs], axis=0)
            y1 = _ln(xres) + st['hs']
            st['y1x'] = xres + y1
            st['h3'] = _dot(_ln(y1).astype(BF16), _ub(w3[...]))

        def mlp_w4():
            st['h4'] = _dot(_gelu(st['h3']).astype(BF16), _ub(w4[...]))

        def mlp_out():
            xnew = st['y1x'] + st['h4']
            st['xnew'] = xnew
            for i, (l, s) in enumerate(rsegs):
                if l == 0:
                    xr[_ds(s, SEG, SEG), :] = xnew[i * SEG:(i + 1) * SEG]
                else:
                    ob[_ds(s, HS, HS), :] = _bu(xnew[i * SEG:(i + 1) * SEG])

        def mlp_send():
            for l, s in rsegs:
                if l == 1:
                    pltpu.make_async_copy(ob.at[_ds(s, HS, HS)], out_u.at[_ds(s, HS, HS)], osem).start()

        slots = {1: (hsegs, mlp_h), 2: (hsegs, mlp_h_store), 3: (rsegs, mlp_w2),
                 NP - 1: (rsegs, mlp_w3), NP: (rsegs, mlp_w4)}

        def mlp_at(key):
            segs, f = slots.get(key, (None, None))
            if segs:
                f()

        if nl == 0:
            for key in sorted(slots):
                mlp_at(key)
            mlp_out()
            mlp_send()
            return

        if first:
            csc[...] = jnp.zeros(csc.shape, F32)
            cv[...] = jnp.zeros(cv.shape, F32)
            cacc[...] = jnp.zeros(cacc.shape, F32)

            def pair_body(p, c_):
                for c in group(p):
                    c.wait()

                @pl.when(p + WIN < NP)
                def _():
                    for c in group(p + WIN):
                        c.start()

                @pl.when(p == NP - 1)
                def _():
                    for c in c_w:
                        c.start()

                q = proj(0, p)
                k = proj(1, p)
                o = values([softmax(csc[:, 0:2 * NK])], cv[...])
                v = proj(2, p)
                cv[...] = v[0:NK]
                csc[:, 0:2 * NK] = scores(q, k)[0]
                cacc[...] += oproj(o, jnp.maximum(p - 1, 0))
                return c_

            lax.fori_loop(0, NP, pair_body, 0)
            acc = cacc[...] + oproj(values([softmax(csc[:, 0:2 * NK])], cv[...]), NP - 1)
        else:
            acc = None
            q = proj(0, 0)
            k = proj(1, 0)
            v = proj(2, 0)
            sc = scores(q, k)
            for p in range(NP):
                mlp_at(p)
                if p + 1 < NP:
                    qn = proj(0, p + 1)
                    kn = proj(1, p + 1)
                prs = [softmax(sc[i]) for i in range(nl)]
                o = values(prs, v)
                if p + 1 < NP:
                    v = proj(2, p + 1)
                    sc = scores(qn, kn)
                else:
                    mlp_at(NP)
                r = oproj(o, p)
                acc = r if acc is None else acc + r
            if rsegs:
                mlp_out()

        if a_on[0]:
            xr[_ds(t, SEG, SEG), :] = xs[0] + acc[0:SEG]
        if a_on[1]:
            i = layers.index(1)
            xr[_ds(t - LAG, SEG, SEG), :] = xs[i] + acc[i * SEG:(i + 1) * SEG]
        if nxt is not None:
            tn = min(t + 1, NSEG - 1) if isinstance(t, int) else jnp.minimum(t + 1, NSEG - 1)
            if nxt == 'layer0':
                lhsf[0:SEG, :] = _ln(x_rows(tn))
            elif nxt == 'layer1':
                lhsf[0:SEG, :] = _ln(st['xnew'][0:SEG])
            else:
                put(lhs, 0, _ln(x_rows(tn)))
                put(lhs, SEG, _ln(st['xnew'][0:SEG]))
        if mem_out:
            if nl == 2:
                mm = acc[nx:]
            elif layers[0] == 0:
                mm = jnp.concatenate([acc[nx:], m0], axis=0)
            else:
                mm = jnp.concatenate([m0, acc[nx:]], axis=0)
            put(lhs, 2 * SEG, mm)
        mlp_send()

    def mlp_segs(t):
        hs = [(l, t - 1 - LAG * l) for l in range(2)]
        rs = [(l, t - 2 - LAG * l) for l in range(2)]
        if isinstance(t, int):
            hs = [(l, s) for l, s in hs if 0 <= s < NSEG]
            rs = [(l, s) for l, s in rs if 0 <= s < NSEG]
        return hs, rs

    BOTH, L0, L1 = (True, True), (True, False), (False, True)

    step(0, L0, *mlp_segs(0), nxt='layer0', first=True)
    c_w[0].wait()
    step(1, L0, *mlp_segs(1), nxt='layer0')
    c_w[1].wait()
    c_w[2].wait()
    c_w[3].wait()
    step(2, L0, *mlp_segs(2), nxt='both')
    step(LAG, BOTH, *mlp_segs(LAG), nxt='both', use_pre=True)
    step(LAG + 1, BOTH, *mlp_segs(LAG + 1), nxt='both', use_pre=True)

    def loop(lo, hi, **kw):
        def body(t, c):
            step(t, BOTH, *mlp_segs(t), nxt='both', **kw)
            return c
        lax.fori_loop(lo, hi, body, 0)

    c_x1.start()
    loop(LAG + 2, LAG + NPRE, use_pre=True)
    c_x1.wait()
    loop(LAG + NPRE, NSEG)
    t = NSEG
    hs, rs = mlp_segs(t)
    lhsf[0:SEG, :] = _ln(xr[_ds(t - LAG, SEG, SEG), :])
    step(t, L1, hs, rs, nxt='layer1')
    step(t + 1, L1, *mlp_segs(t + 1), nxt='layer1')
    step(t + 2, L1, *mlp_segs(t + 2), mem_out=False)
    step(t + 3, (False, False), [(1, NSEG - 1)], [(1, NSEG - 2), (1, NSEG - 1)])
    pltpu.make_async_copy(ob, out_u, osem).wait()


def _call(A_x, A_mem0, A_Wq, A_Wk, A_Wv, A_Wo, B_w1, B_w2, B_w3, B_w4):
    x = A_x.reshape(S, D)
    mem0 = A_mem0.reshape(M, D)
    tr = lambda w: jnp.transpose(w, (1, 2, 0)).reshape(HD, D)
    hbm = pl.BlockSpec(memory_space=pltpu.HBM)
    out = pl.pallas_call(
        _kernel,
        out_shape=jax.ShapeDtypeStruct((S, D), BF16),
        in_specs=[hbm] * 10,
        out_specs=hbm,
        scratch_shapes=[
            pltpu.VMEM((S // 2, D), U32),
            pltpu.VMEM((M, D), BF16),
            pltpu.VMEM((HD // 2, D), U32),
            pltpu.VMEM((HD // 2, D), U32),
            pltpu.VMEM((HD // 2, D), U32),
            pltpu.VMEM((HD // 2, D), U32),
            pltpu.VMEM((D // 2, D), U32),
            pltpu.VMEM((D // 2, D), U32),
            pltpu.VMEM((D // 2, FF), U32),
            pltpu.VMEM((FF // 2, D), U32),
            pltpu.VMEM((S, D), F32),
            pltpu.VMEM((2, S + 2 * HALO, D), F32),
            pltpu.VMEM((S // 2, D), U32),
            pltpu.VMEM((SEG + M, D), U32),
            pltpu.VMEM(((NPRE * PRE_ROWS + SEG + 2 * M) // 2, D), U32),
            pltpu.VMEM((SEG + M, D), F32),
            pltpu.VMEM((3, NP, NPRE * PRE_ROWS // 2, PW), U32),
            pltpu.VMEM((3, NP, D // 2, PW), U32),
            pltpu.VMEM((SEG + M, 128), F32),
            pltpu.VMEM((SEG + M, PW), F32),
            pltpu.VMEM((SEG + M, D), F32),
            pltpu.SemaphoreType.DMA((7,)),
            pltpu.SemaphoreType.DMA((NP,)),
            pltpu.SemaphoreType.DMA,
        ],
        compiler_params=pltpu.CompilerParams(vmem_limit_bytes=110 * 1024 * 1024),
    )(x, mem0, tr(A_Wq), tr(A_Wk), tr(A_Wv), A_Wo.reshape(HD, D), B_w1, B_w2, B_w3, B_w4)
    return out.reshape(1, S, D)


@functools.partial(jax.jit, static_argnames=["A_seg_len"])
def pallas_interleave_layers__memory_aug_recurrent_mem_tr__mixer_s_mlp__prompt_kernel(
        A_x, A_mem0, A_Wq, A_Wk, A_Wv, A_Wo, A_seg_len, B_x, B_w1, B_w2, B_w3, B_w4):
    assert A_seg_len == SEG and A_x.shape == (1, S, D) and A_Wq.shape == (D, H, DH)
    assert A_mem0.shape == (1, M, D) and B_w3.shape == (D, FF)
    del B_x
    return _call(A_x, A_mem0, A_Wq, A_Wk, A_Wv, A_Wo, B_w1, B_w2, B_w3, B_w4)
```
